```python
import jax
import jax.numpy as jnp

def _softmax(x, axis=-1):
    return jax.nn.softmax(x, axis=axis)

def _gelu(x):
    return jax.nn.gelu(x, approximate=True)

def _silu(x):
    return jax.nn.silu(x)

def _sigmoid(x):
    return jax.nn.sigmoid(x)

def _layernorm(x, axis=-1, eps=1e-05):
    m = jnp.mean(x, axis=axis, keepdims=True)
    v = jnp.var(x, axis=axis, keepdims=True)
    return (x - m) / jnp.sqrt(v + eps)

def _scatter_add(tgt, idx, src, axis=0):
    return tgt.at[idx].add(src)

def _segment_sum(src, seg, n):
    return jax.ops.segment_sum(src, seg, n)

class _Rng:

    def __init__(self, key):
        self._k = key

    def _next(self):
        self._k, sub = jax.random.split(self._k)
        return sub

    def normal(self, shape):
        return jax.random.normal(self._next(), shape, dtype=jnp.bfloat16)

    def randint(self, lo, hi, shape):
        return jax.random.randint(self._next(), shape, lo, hi, dtype=jnp.int32)

    def uniform(self, shape, lo=0.0, hi=1.0):
        return jax.random.uniform(self._next(), shape, jnp.bfloat16, lo, hi)

    def permutation(self, n):
        return jax.random.permutation(self._next(), n)
kernel_name = 'adaLN_cond__ssm_conv_h3__glu_gated_bilinear__prompt'

def setup_inputs():
    _rng = _Rng(jax.random.key(int.from_bytes(__import__("os").urandom(4), "little")))
    _w = lambda a: (lambda t: t.astype(jnp.bfloat16) if jnp.issubdtype(t.dtype, jnp.floating) else t)(jnp.asarray(a))

    def _A_setup():
        B, S, D = (1, 2048, 640)
        ks = 4
        return {'q': _w((lambda *s: _rng.normal(s) * 0.05)(B, S, D)), 'k': _w((lambda *s: _rng.normal(s) * 0.05)(B, S, D)), 'v': _w((lambda *s: _rng.normal(s) * 0.05)(B, S, D)), 'shift_k': _w((lambda *s: _rng.normal(s) * 0.05)(D, ks) * 0.5), 'ssm_k': _w((lambda *s: _rng.normal(s) * 0.05)(D, S) * (1.0 / S ** 0.5)), 'ssm_D': _w((lambda *s: _rng.normal(s) * 0.05)(D))}
    _A_in = _A_setup()

    def _B_setup():
        B, S, D, F = (1, 2048, 640, 1536)
        return {'x': _w((lambda *s: _rng.normal(s) * 0.05)(B, S, D)), 'w_gate': _w((lambda *s: _rng.normal(s) * 0.05)(D, F) * D ** (-0.5)), 'w_up': _w((lambda *s: _rng.normal(s) * 0.05)(D, F) * D ** (-0.5)), 'w_down': _w((lambda *s: _rng.normal(s) * 0.05)(F, D) * F ** (-0.5))}
    _B_in = _B_setup()
    return {'A_q': _A_in['q'], 'A_k': _A_in['k'], 'A_v': _A_in['v'], 'A_shift_k': _A_in['shift_k'], 'A_ssm_k': _A_in['ssm_k'], 'A_ssm_D': _A_in['ssm_D'], 'B_x': _B_in['x'], 'B_w_gate': _B_in['w_gate'], 'B_w_up': _B_in['w_up'], 'B_w_down': _B_in['w_down'], 'c': _w((lambda *s: _rng.normal(s) * 0.05)(1, 640)), 'w_mod': _w((lambda *s: _rng.normal(s) * 0.05)(640, 6 * 640) * 640 ** (-0.5))}

def reference(A_q, A_k, A_v, A_shift_k, A_ssm_k, A_ssm_D, B_x, B_w_gate, B_w_up, B_w_down, c, w_mod):

    def _A_ref(q, k, v, shift_k, ssm_k, ssm_D):
        B, S, D = q.shape
        ks = shift_k.shape[-1]
        k_pad = jnp.pad(k, ((0, 0), (ks - 1, 0), (0, 0)))
        k_shift = jnp.zeros_like(k)
        for t in range(ks):
            k_shift = k_shift + k_pad[:, t:t + S, :] * shift_k[:, ks - 1 - t][None, None, :]
        kv = k_shift * v
        L = 2 * S
        kv_pad = jnp.pad(kv, ((0, 0), (0, S), (0, 0)))
        kf_pad = jnp.pad(ssm_k, ((0, 0), (0, S)))
        kv_f = (lambda x, axes=(-2, -1): jnp.fft.rfft2(x.astype(jnp.float32), axes=axes))(kv_pad[:, None, :, :], axes=(1, 2))
        kf_f = (lambda x, axes=(-2, -1): jnp.fft.rfft2(x.astype(jnp.float32), axes=axes))(kf_pad[:, None, :], axes=(1, 2))
        kf_f = (lambda x, *d: x.transpose(*d))(kf_f, 1, 2, 0)
        y_f = kv_f * kf_f[None, :, :, :]
        y = (lambda x, s, axes=(-2, -1): jnp.fft.irfft2(x, s=s, axes=axes).astype(jnp.bfloat16))(y_f, (1, L), axes=(1, 2))[:, 0, :S, :]
        y = y + kv * ssm_D[None, None, :]
        return q * y

    def _B_ref(x, w_gate, w_up, w_down):
        g = jnp.einsum('bsd,df->bsf', x, w_gate)
        u = jnp.einsum('bsd,df->bsf', x, w_up)
        h = g * u
        return jnp.einsum('bsf,fd->bsd', h, w_down)
    x = A_q
    mod = (_silu(c) @ w_mod).reshape(c.shape[0], 6, 1, -1)
    sa, ca, ga, sb, cb, gb = (mod[:, 0].copy(), mod[:, 1].copy(), mod[:, 2].copy(), mod[:, 3].copy(), mod[:, 4].copy(), mod[:, 5].copy())
    h = _layernorm(x, axis=-1) * (1 + ca) + sa
    x = x + ga * _A_ref(h, A_k, A_v, A_shift_k, A_ssm_k, A_ssm_D)
    h = _layernorm(x, axis=-1) * (1 + cb) + sb
    x = x + gb * _B_ref(h, B_w_gate, B_w_up, B_w_down)
    return x
```

```python
import functools
import numpy as np
import jax
import jax.numpy as jnp
from jax import lax
from jax.experimental import pallas as pl
from jax.experimental.pallas import tpu as pltpu

S, D, F = 2048, 640, 1536
T = 128
NB = S // T
H = T // 2
EPS = 1e-5
bf16 = jnp.bfloat16
f32 = jnp.float32


def _dft_consts():
    n = np.arange(T)
    f = np.concatenate([np.arange(0, T, 2), np.arange(1, T, 2)])
    ph = ((2 * f[:, None] + 1) * n[None, :]) % (4 * T)
    ang = 2.0 * np.pi * ph / (4 * T)
    c_, s_ = np.cos(ang).reshape(T // 8, 8, T), -np.sin(ang).reshape(T // 8, 8, T)
    fwd = np.concatenate([c_, s_], axis=1).reshape(2 * T, T)
    inv = fwd.T / T
    return fwd.astype(np.float32).astype(bf16), inv.astype(np.float32).astype(bf16)


def make_kernel(interpret=False, TM=256, WC=512, units=None, vmem_mb=100, flags=None,
                t_kv=(0, 1500), t_us=4, t_m=(0, 800), n_inv=2, t_e=(1, 400), t_ks=-1, nslot_g=10, nslot_d=32, inj='lhs', kstep=2, force_inj=False):
    R = TM // T
    NM = S // TM
    NT = 128
    NGU = F // NT
    NDN = D // NT
    NWC = F // WC

    def kernel(q_hbm, k_hbm, v_hbm, shift_hbm, ssmk_hbm, ssmd_hbm, wg_hbm, wu_hbm, wd_hbm, c_hbm, wmod_hbm,
               ft_hbm, g_hbm, zero_smem, out_hbm,
               q_v, k_v, v_v, shift_v, ssmk_v, ssmd_v, wg_v, wu_v, wd_v, c_v, wmod_v, ft_v, g_v,
               sp_v, kraw_v, kv_v, z_v, y_v, h2_v, x1_v, out_v, mod_v, par_v, hh_v, sems):
        never = zero_smem[0] > 0

        plan = []

        def add(name, src, dst):
            plan.append((name, src, dst))

        def rows(m):
            return slice(m * TM, (m + 1) * TM)

        def add_kv(m):
            add(("k", m), k_hbm.at[rows(m)], k_v.at[rows(m)])
            add(("v", m), v_hbm.at[rows(m)], v_v.at[rows(m)])

        def add_s(m):
            add(("ssmk", m), ssmk_hbm.at[:, rows(m)], ssmk_v.at[:, rows(m)])

        def add_q(m):
            add(("q", m), q_hbm.at[rows(m)], q_v.at[rows(m)])

        def add_w(c):
            cols = slice(c * WC, (c + 1) * WC)
            add(("wg", c), wg_hbm.at[:, cols], wg_v.at[:, cols])
            add(("wu", c), wu_hbm.at[:, cols], wu_v.at[:, cols])

        add("ft", ft_hbm, ft_v)
        add("shift", shift_hbm, shift_v)
        add_kv(0); add_s(0)
        add("g", g_hbm, g_v)
        add("c", c_hbm, c_v)
        add("ssmd", ssmd_hbm, ssmd_v)
        add("wmod_a", wmod_hbm.at[:, 0:3 * D], wmod_v.at[:, 0:3 * D])
        add_q(0)
        add("wmod_b", wmod_hbm.at[:, 3 * D:5 * D], wmod_v.at[:, 3 * D:5 * D])
        add_w(0)
        add_kv(1); add_s(1)
        add_w(1)
        add_q(1)
        add_w(2)
        add_kv(2); add_s(2)
        add("wd", wd_hbm, wd_v)
        add("wmod_c", wmod_hbm.at[:, 5 * D:6 * D], wmod_v.at[:, 5 * D:6 * D])
        add_q(2)
        for m in range(3, NM):
            add_kv(m); add_s(m); add_q(m)
        cps = {}
        for i, (name, src, dst) in enumerate(plan):
            cps[name] = pltpu.make_async_copy(src, dst, sems.at[i])
        n_in = len(plan)
        for name, _, _ in plan:
            cps[name].start()
        waited = set()

        def wait(*names):
            for name in names:
                if name not in waited:
                    waited.add(name)
                    cps[name].wait()

        def kspec(d):
            kblk = ssmk_v[:, d * T:(d + 1) * T]
            raw = lax.dot_general(ft_v[...], kblk, (((1,), (1,)), ((), ())), preferred_element_type=f32)
            if d == 0:
                sp_v[NB] = raw
            else:
                p = (d - 1) % 2
                for g in range(T // 8):
                    re = slice(16 * g, 16 * g + 8)
                    im = slice(16 * g + 8, 16 * g + 16)
                    if g < T // 16:
                        sp_v[NB + d, re, :] = raw[re] - kraw_v[p, im, :]
                        sp_v[NB + d, im, :] = raw[im] + kraw_v[p, re, :]
                    else:
                        sp_v[NB + d, re, :] = raw[re] + kraw_v[p, im, :]
                        sp_v[NB + d, im, :] = raw[im] - kraw_v[p, re, :]
            if d < NB - 1:
                kraw_v[d % 2] = raw

        def uspec(j):
            sp_v[j] = jnp.dot(ft_v[...], kv_v[j * T:(j + 1) * T, :], preferred_element_type=f32)

        def kv_piece(r0):
            kc = k_v[r0:r0 + 16, :].astype(f32)
            if r0 == 0:
                kp = jnp.zeros((8, D), f32)
            else:
                kp = k_v[r0 - 16:r0, :].astype(f32)[8:16]
            ext = jnp.concatenate([kp, kc], axis=0)
            ks = kc * par_v[0, 0:1, :]
            for t in range(1, 4):
                ks = ks + ext[8 - t:24 - t] * par_v[t, 0:1, :]
            kv = (ks * v_v[r0:r0 + 16, :].astype(f32)).astype(bf16)
            kv_v[r0:r0 + 16, :] = kv
            return [kv[:, c * 128:(c + 1) * 128] for c in range(5)]

        def mac_piece(i, r, c):
            zb = i % (2 * R)
            re = slice(r * 16, r * 16 + 8)
            im = slice(r * 16 + 8, r * 16 + 16)
            cs = slice(c * 128, (c + 1) * 128)
            ar = ai = None
            for j in range(i + 1):
                kr = sp_v[NB + i - j, re, cs]
                ki = sp_v[NB + i - j, im, cs]
                ur = sp_v[j, re, cs]
                ui = sp_v[j, im, cs]
                tr = kr * ur - ki * ui
                ti = kr * ui + ki * ur
                ar = tr if ar is None else ar + tr
                ai = ti if ai is None else ai + ti
            z = jnp.concatenate([ar, ai], axis=0).astype(bf16)
            z_v[zb, r * 16:r * 16 + 16, cs] = z
            return [z]

        def inv(i):
            y_v[i % (2 * R)] = jnp.dot(g_v[...], z_v[i % (2 * R)], preferred_element_type=f32)

        def stats(x):
            m = jnp.sum(x, axis=-1, keepdims=True) * (1.0 / D)
            xc = x - m
            var = jnp.sum(xc * xc, axis=-1, keepdims=True) * (1.0 / D)
            return xc * lax.rsqrt(var + EPS)

        def epi_piece(r0):
            i = r0 // T
            rs = slice(r0, r0 + 16)
            y = y_v[i % (2 * R), r0 - i * T:r0 - i * T + 16, :] + kv_v[rs, :].astype(f32) * par_v[4, 0:1, :]
            x = q_v[rs, :].astype(f32)
            x1 = x + (stats(x) * mod_v[0, 0:1, :] + mod_v[1, 0:1, :]) * y
            h2 = (stats(x1) * mod_v[2, 0:1, :] + mod_v[3, 0:1, :]).astype(bf16)
            x1_v[rs, :] = x1
            h2_v[rs, :] = h2
            return [h2[:, c * 128:(c + 1) * 128] for c in range(5)]

        def params():
            sh = shift_v[...].astype(f32)
            for t in range(4):
                par_v[t] = jnp.broadcast_to(sh[t:t + 1, :], (8, D))
            par_v[4] = jnp.broadcast_to(ssmd_v[...].astype(f32).reshape(1, D), (8, D))

        def mods(lo, hi):
            cc = c_v[...].astype(f32)
            sc = (cc * jax.nn.sigmoid(cc)).astype(bf16)
            sc = jnp.broadcast_to(sc, (16, D))
            md = [jnp.dot(sc, wmod_v[:, i * D:(i + 1) * D], preferred_element_type=f32)[0:8, :] for i in range(lo, hi)]
            return md

        def mods_a():
            sa, ca, ga = mods(0, 3)
            mod_v[0] = ga * (1.0 + ca)
            mod_v[1] = ga * sa

        def mods_b():
            sb, cb = mods(3, 5)
            mod_v[2] = 1.0 + cb
            mod_v[3] = sb

        def mods_c():
            (gb,) = mods(5, 6)
            mod_v[4] = gb

        koff = [0]

        def dot_w(lhs, rhs, thunks):
            toks = []
            for th in thunks:
                toks.extend(th())
            if interpret and not force_inj:
                toks = []
            if toks and inj == "lhs":
                M_, K = lhs.shape
                nr, nk = M_ // 16, K // 128
                n = len(toks)
                cells = {}
                for j, t_ in enumerate(toks):
                    rr = (j * nr) // n if n <= nr else j % nr
                    kt = (j * kstep + koff[0]) % nk
                    while (rr, kt) in cells:
                        kt = (kt + 1) % nk
                    cells[(rr, kt)] = t_
                koff[0] += 1
                rowp = []
                for rr in range(nr):
                    cols_ = []
                    for kt in range(nk):
                        base = lhs[rr * 16:(rr + 1) * 16, kt * 128:(kt + 1) * 128]
                        cols_.append(jnp.where(never, cells[(rr, kt)], base) if (rr, kt) in cells else base)
                    rowp.append(jnp.concatenate(cols_, axis=1))
                lhs = jnp.concatenate(rowp, axis=0)
            elif toks:
                K = rhs.shape[0]
                nsl = K // 16
                assert len(toks) <= nsl, (len(toks), nsl)
                pos = [(i * nsl) // len(toks) for i in range(len(toks))]
                parts = []
                prev = 0
                for p_, t_ in zip(pos, toks):
                    r0 = p_ * 16
                    if r0 > prev:
                        parts.append(rhs[prev:r0])
                    parts.append(jnp.where(never, t_, rhs[r0:r0 + 16]))
                    prev = r0 + 16
                if prev < K:
                    parts.append(rhs[prev:])
                rhs = jnp.concatenate(parts, axis=0)
            return jnp.dot(lhs, rhs, preferred_element_type=f32)

        wait("ft", "shift", "ssmd", ("k", 0), ("v", 0))
        params()
        for r0 in range(0, TM, 16):
            kv_piece(r0)
        wait(("ssmk", 0))
        for b in range(R):
            kspec(b)
            uspec(b)
        wait("g")
        for b in range(R):
            for r in range(T // 8):
                for c in range(5):
                    mac_piece(b, r, c)
            inv(b)
        wait("c", "wmod_a", ("q", 0))
        mods_a()
        wait("wmod_b")
        mods_b()
        for r0 in range(0, TM, 16):
            epi_piece(r0)

        def out_copy(m):
            return pltpu.make_async_copy(out_v.at[rows(m), :], out_hbm.at[rows(m), :], sems.at[n_in + m])

        GU_T = 5 * TM // 4
        DN_T = (F // 128) * TM // 4
        SP_T = 5 * 256 // 4

        for m in (range(NM) if units is None else units):
            m1 = m + 1
            m2 = m + 2
            ev = []
            if m2 < NM and m > 0:
                ev += [("ks", b, SP_T) for b in range(m2 * R, (m2 + 1) * R)]
            for n in range(NGU):
                ev.append(("g", n, GU_T)); ev.append(("u", n, GU_T))
                if n == t_us and m2 < NM and m > 0:
                    ev += [("us", b, SP_T) for b in range(m2 * R, (m2 + 1) * R)]
            for n in range(NDN):
                ev.append(("d", n, DN_T))
                if n + 1 == n_inv and m1 < NM and m > 0:
                    ev += [("inv", b, SP_T) for b in range(m1 * R, (m1 + 1) * R)]
            tt = 0
            starts = []
            for e in ev:
                starts.append(tt); tt += e[2]
            t_end = tt
            streams = []
            if m > 0:
                if m2 < NM:
                    t_us_ = [starts[i] for i, e in enumerate(ev) if e[0] == "us"][0]
                    streams.append(([functools.partial(kv_piece, r0) for r0 in range(m2 * TM, (m2 + 1) * TM, 16)], [5] * 16, (0, t_us_ - 2 * GU_T)))
                if m1 < NM:
                    t_inv_ = [starts[i] for i, e in enumerate(ev) if e[0] == "inv"][0]
                    streams.append(([functools.partial(mac_piece, b, r, c) for b in range(m1 * R, (m1 + 1) * R)
                                     for r in range(T // 8) for c in range(5)], [1] * (R * 80), (t_m[0], t_inv_ - t_m[1])))
                    streams.append(([functools.partial(epi_piece, r0) for r0 in range(m1 * TM, (m1 + 1) * TM, 16)], [5] * 16,
                                    (t_inv_ + 2 * SP_T + t_e[0], t_end - t_e[1])))
            if m > 0:
                out_copy(m - 1).start()
                if m2 < NM:
                    wait(("k", m2), ("v", m2), ("ssmk", m2))
                if m1 < NM:
                    wait(("q", m1))
            assign = {i: [] for i in range(len(ev))}
            cap = {i: (nslot_g if e[0] in "gu" else nslot_d if e[0] == "d" else 0) for i, e in enumerate(ev)}
            for thunks, ntok, (ta, tb) in streams:
                n = len(thunks)
                for p_, th in enumerate(thunks):
                    tp = ta + (tb - ta) * p_ / n
                    cand = [i for i, e in enumerate(ev) if cap[i] >= ntok[p_] and starts[i] + e[2] > tp]
                    i = cand[0]
                    assign[i].append(th); cap[i] -= ntok[p_]

            hh_parts = {}
            gval = None
            for i, (kind, n, _) in enumerate(ev):
                if kind == "ks":
                    kspec(n)
                elif kind == "us":
                    uspec(n)
                elif kind == "inv":
                    inv(n)
                elif kind == "g":
                    cols = slice(n * NT, (n + 1) * NT)
                    if m == 0 and (n * NT) % WC == 0:
                        cc_ = n * NT // WC
                        wait(("wg", cc_), ("wu", cc_))
                        if cc_ == 1:
                            wait(("k", 1), ("v", 1), ("ssmk", 1))
                            for r0 in range(TM, 2 * TM, 16):
                                kv_piece(r0)
                            for b in range(R, 2 * R):
                                kspec(b); uspec(b)
                        if cc_ == 2:
                            wait(("q", 1))
                            for b in range(R, 2 * R):
                                for r in range(T // 8):
                                    for c in range(5):
                                        mac_piece(b, r, c)
                                inv(b)
                            for r0 in range(TM, 2 * TM, 16):
                                epi_piece(r0)
                    gval = dot_w(h2_v[rows(m), :], wg_v[:, cols], assign[i])
                elif kind == "u":
                    cols = slice(n * NT, (n + 1) * NT)
                    uval = dot_w(h2_v[rows(m), :], wu_v[:, cols], assign[i])
                    hh_v[:, cols] = (gval * uval).astype(bf16)
                elif kind == "d":
                    cols = slice(n * NT, (n + 1) * NT)
                    if m == 0 and n == 0:
                        wait("wd", "wmod_c", ("k", 2), ("v", 2), ("ssmk", 2))
                        mods_c()
                        for r0 in range(2 * TM, 3 * TM, 16):
                            kv_piece(r0)
                        for b in range(2 * R, 3 * R):
                            kspec(b); uspec(b)
                    p = dot_w(hh_v[...], wd_v[:, cols], assign[i])
                    out_v[rows(m), cols] = (x1_v[rows(m), cols] + mod_v[4, 0:1, cols] * p).astype(bf16)
        ms = list(range(NM) if units is None else units)
        out_copy(ms[-1]).start()
        for m in ms:
            if m == ms[-1] or (m + 1) in ms:
                out_copy(m).wait()
        for name, _, _ in plan:
            wait(name)

    def run(A_q, A_k, A_v, A_shift_k, A_ssm_k, A_ssm_D, B_x, B_w_gate, B_w_up, B_w_down, c, w_mod):
        ft, g = _dft_consts()
        any_ = pl.BlockSpec(memory_space=pl.ANY)
        V = pltpu.VMEM
        nsem = 12 + 4 * NM + 2 * NWC + NM
        out = pl.pallas_call(
            kernel,
            out_shape=jax.ShapeDtypeStruct((S, D), bf16),
            in_specs=[any_] * 13 + [pl.BlockSpec(memory_space=pltpu.SMEM)],
            out_specs=any_,
            scratch_shapes=[
                V((S, D), bf16), V((S, D), bf16), V((S, D), bf16), V((4, D), bf16), V((D, S), bf16), V((D,), bf16),
                V((D, F), bf16), V((D, F), bf16), V((F, D), bf16), V((1, D), bf16), V((D, 6 * D), bf16),
                V((2 * T, T), bf16), V((T, 2 * T), bf16),
                V((2 * NB, 2 * T, D), f32), V((2, 2 * T, D), f32), V((S, D), bf16),
                V((2 * R, 2 * T, D), bf16), V((2 * R, T, D), f32), V((S, D), bf16), V((S, D), f32),
                V((S, D), bf16), V((5, 8, D), f32), V((5, 8, D), f32), V((TM, F), bf16),
                pltpu.SemaphoreType.DMA((nsem,)),
            ],
            compiler_params=pltpu.CompilerParams(vmem_limit_bytes=vmem_mb * 1024 * 1024, flags=flags),
            interpret=interpret,
        )(A_q.reshape(S, D), A_k.reshape(S, D), A_v.reshape(S, D), A_shift_k.T, A_ssm_k, A_ssm_D,
          B_w_gate, B_w_up, B_w_down, c, w_mod, ft, g, np.zeros((1,), np.int32))
        return out.reshape(1, S, D)
    return run


_run = make_kernel(nslot_g=16)


@jax.jit
def pallas_adaLN_cond__ssm_conv_h3__glu_gated_bilinear__prompt_kernel(
    A_q: jax.Array,
    A_k: jax.Array,
    A_v: jax.Array,
    A_shift_k: jax.Array,
    A_ssm_k: jax.Array,
    A_ssm_D: jax.Array,
    B_x: jax.Array,
    B_w_gate: jax.Array,
    B_w_up: jax.Array,
    B_w_down: jax.Array,
    c: jax.Array,
    w_mod: jax.Array,
):
    return _run(A_q, A_k, A_v, A_shift_k, A_ssm_k, A_ssm_D, B_x, B_w_gate, B_w_up, B_w_down, c, w_mod)
```

```python
import functools
import numpy as np
import jax
import jax.numpy as jnp
from jax import lax
from jax.experimental import pallas as pl
from jax.experimental.pallas import tpu as pltpu

S, D, F = 2048, 640, 1536
T = 128
NB = S // T
H = T // 2
EPS = 1e-5
bf16 = jnp.bfloat16
f32 = jnp.float32


def _dft_consts():
    n = np.arange(T)
    f = np.concatenate([np.arange(0, T, 2), np.arange(1, T, 2)])
    ph = ((2 * f[:, None] + 1) * n[None, :]) % (4 * T)
    ang = 2.0 * np.pi * ph / (4 * T)
    c_, s_ = np.cos(ang).reshape(T // 8, 8, T), -np.sin(ang).reshape(T // 8, 8, T)
    fwd = np.concatenate([c_, s_], axis=1).reshape(2 * T, T)
    inv = fwd.T / T
    return fwd.astype(np.float32).astype(bf16), inv.astype(np.float32).astype(bf16)


def make_kernel(interpret=False, TM=256, WCH=(0, 1, 4, 8, 12), DCH=(0, 2, 4, 5), units=None, vmem_mb=100, flags=None,
                t_kv=(0, 1500), t_us=4, t_m=(0, 500), n_inv=2, t_e=(1, 400), t_ks=-1, nslot_g=60, nslot_d=100, inj='lhs', kstep=2, force_inj=False, pre_n0=2, dbg_waitall=False, merge=(), KSP=3, do_pace=True, pace_w=(200, 1200), yval=True, ew=(60., 150., 70.), w_kv1=3500, w_e1=7000, mk_ov=1.0, tps=5, lag=2, bsel=True, scopes=False):
    R = TM // T
    NM = S // TM
    NT = 128
    NGU = F // NT
    NDN = D // NT
    NWC = len(WCH) - 1

    def kernel(q_hbm, k_hbm, v_hbm, shift_hbm, ssmk_hbm, ssmd_hbm, wg_hbm, wu_hbm, wd_hbm, c_hbm, wmod_hbm,
               ft_hbm, g_hbm, zero_smem, out_hbm,
               q_v, k_v, v_v, shift_v, ssmk_v, ssmd_v, wg_v, wu_v, wd_v, c_v, wmod_v, ft_v, g_v,
               sp_v, kraw_v, kv_v, z_v, y_v, h2_v, x1_v, out_v, mod_v, par_v, hh_v, sems):
        never = zero_smem[0] > 0

        plan = []

        def add(name, src, dst):
            plan.append((name, src, dst))

        def rows(m):
            return slice(m * TM, (m + 1) * TM)

        def add_kv(m):
            add(("k", m), k_hbm.at[rows(m)], k_v.at[rows(m)])
            add(("v", m), v_hbm.at[rows(m)], v_v.at[rows(m)])

        def add_s(m):
            add(("ssmk", m), ssmk_hbm.at[:, rows(m)], ssmk_v.at[:, rows(m)])

        def add_q(m):
            add(("q", m), q_hbm.at[rows(m)], q_v.at[rows(m)])

        def add_w(c):
            cols = slice(WCH[c] * NT, WCH[c + 1] * NT)
            add(("wg", c), wg_hbm.at[:, cols], wg_v.at[:, cols])
            add(("wu", c), wu_hbm.at[:, cols], wu_v.at[:, cols])

        def add_wd(c):
            cols = slice(DCH[c] * NT, DCH[c + 1] * NT)
            add(("wd", c), wd_hbm.at[:, cols], wd_v.at[:, cols])

        add("ft", ft_hbm, ft_v)
        add("shift", shift_hbm, shift_v)
        add("ssmd", ssmd_hbm, ssmd_v)
        add_kv(0); add_s(0)
        add("g", g_hbm, g_v)
        add("c", c_hbm, c_v)
        add("wmod_a", wmod_hbm.at[:, 0:3 * D], wmod_v.at[:, 0:3 * D])
        add_q(0)
        add("wmod_b", wmod_hbm.at[:, 3 * D:5 * D], wmod_v.at[:, 3 * D:5 * D])
        add_w(0); add_w(1); add_w(2)
        add_kv(1); add_s(1); add_w(3)
        add_q(1)
        add_wd(0)
        add("wmod_c", wmod_hbm.at[:, 5 * D:6 * D], wmod_v.at[:, 5 * D:6 * D])
        add_wd(1); add_wd(2)
        for m in range(2, NM):
            add_kv(m); add_s(m); add_q(m)
        cps = {}
        for i, (name, src, dst) in enumerate(plan):
            cps[name] = pltpu.make_async_copy(src, dst, sems.at[i])
        n_in = len(plan)
        for name, _, _ in plan:
            cps[name].start()
        waited = set()

        def wait(*names):
            for name in names:
                if name not in waited:
                    waited.add(name)
                    if scopes:
                        with jax.named_scope("w_" + "_".join(map(str, name)) if isinstance(name, tuple) else "w_" + name):
                            cps[name].wait()
                    else:
                        cps[name].wait()

        if dbg_waitall:
            for name, _, _ in plan:
                wait(name)
            units_ = []
        def i32(x):
            return pltpu.bitcast(x, jnp.int32)

        def toks16(x):
            xi = i32(x[0:8]) ^ i32(x[8:16])
            return [xi[:, c * 128:(c + 1) * 128] for c in range(5)]

        def kspec(d):
            kblk = ssmk_v[:, d * T:(d + 1) * T]
            raw = lax.dot_general(ft_v[...], kblk, (((1,), (1,)), ((), ())), preferred_element_type=f32)
            if d == 0:
                sp_v[NB] = raw
            else:
                p = (d - 1) % 2
                for g in range(T // 8):
                    re = slice(16 * g, 16 * g + 8)
                    im = slice(16 * g + 8, 16 * g + 16)
                    if g < T // 16:
                        sp_v[NB + d, re, :] = raw[re] - kraw_v[p, im, :]
                        sp_v[NB + d, im, :] = raw[im] + kraw_v[p, re, :]
                    else:
                        sp_v[NB + d, re, :] = raw[re] + kraw_v[p, im, :]
                        sp_v[NB + d, im, :] = raw[im] - kraw_v[p, re, :]
            if d < NB - 1:
                kraw_v[d % 2] = raw

        def uspec(j):
            sp_v[j] = jnp.dot(ft_v[...], kv_v[j * T:(j + 1) * T, :], preferred_element_type=f32)

        def kv_piece(r0):
            kc = k_v[r0:r0 + 16, :].astype(f32)
            if r0 == 0:
                kp = jnp.zeros((8, D), f32)
            else:
                kp = k_v[r0 - 16:r0, :].astype(f32)[8:16]
            ext = jnp.concatenate([kp, kc], axis=0)
            ks = kc * par_v[0, 0:1, :]
            for t in range(1, 4):
                ks = ks + ext[8 - t:24 - t] * par_v[t, 0:1, :]
            kvf = ks * v_v[r0:r0 + 16, :].astype(f32)
            kv_v[r0:r0 + 16, :] = kvf.astype(bf16)
            return toks16(kvf)

        memo = {}
        pace = {}

        def mac_piece(i, r, c, cuts=None, k_=None):
            if cuts is None:
                cuts, k_ = (0, i + 1), 0
            key = ("mac", i, r, c, k_)
            if key in memo:
                return memo[key][2]
            zb = i % (2 * R)
            re = slice(r * 16, r * 16 + 8)
            im = slice(r * 16 + 8, r * 16 + 16)
            cs = slice(c * 128, (c + 1) * 128)
            ar = ai = None
            if k_ > 0:
                mac_piece(i, r, c, cuts, k_ - 1)
                ar, ai, _ = memo[("mac", i, r, c, k_ - 1)]
            for j in range(cuts[k_], cuts[k_ + 1]):
                kr = sp_v[NB + i - j, re, cs]
                ki = sp_v[NB + i - j, im, cs]
                ur = sp_v[j, re, cs]
                ui = sp_v[j, im, cs]
                tr = kr * ur - ki * ui
                ti = kr * ui + ki * ur
                ar = tr if ar is None else ar + tr
                ai = ti if ai is None else ai + ti
            if cuts[k_ + 1] == i + 1:
                z_v[zb, r * 16:r * 16 + 16, cs] = jnp.concatenate([ar, ai], axis=0).astype(bf16)
            memo[key] = (ar, ai, [i32(ar) ^ i32(ai)])
            return memo[key][2]

        def inv(i):
            yv = jnp.dot(g_v[...], z_v[i % (2 * R)], preferred_element_type=f32)
            if yval:
                memo[("y", i)] = yv
            else:
                y_v[i % (2 * R)] = yv

        def moments(x):
            m = jnp.sum(x, axis=-1, keepdims=True) * (1.0 / D)
            q = jnp.sum(x * x, axis=-1, keepdims=True) * (1.0 / D)
            rstd = lax.rsqrt(jnp.maximum(q - m * m, 0.0) + EPS)
            return m, rstd

        def btok(v):
            vb = jnp.broadcast_to(v, (16, 128))
            return i32(vb[0:8]) ^ i32(vb[8:16])

        def epi_piece(r0, stage=2):
            key = ("epi", r0, stage)
            if key in memo:
                return memo[key][0]
            i = r0 // T
            rs = slice(r0, r0 + 16)
            if stage == 0:
                m, rstd = moments(q_v[rs, :].astype(f32))
                memo[key] = ([btok(rstd) ^ btok(m)], m, rstd)
            elif stage == 1:
                epi_piece(r0, 0)
                _, m, rstd = memo[("epi", r0, 0)]
                if yval:
                    yc = memo[("y", i)][r0 - i * T:r0 - i * T + 16]
                else:
                    yc = y_v[i % (2 * R), r0 - i * T:r0 - i * T + 16, :]
                y = yc + kv_v[rs, :].astype(f32) * par_v[4, 0:1, :]
                if r0 in pace:
                    y = jnp.where(never, jnp.tile(pace.pop(r0), (2, 5)), y)
                x = q_v[rs, :].astype(f32)
                x1 = x + (((x - m) * rstd) * mod_v[0, 0:1, :] + mod_v[1, 0:1, :]) * y
                x1_v[rs, :] = x1
                m2, rstd2 = moments(x1)
                memo[key] = ([btok(rstd2) ^ btok(m2)], x1, m2, rstd2)
            else:
                epi_piece(r0, 1)
                _, x1, m2, rstd2 = memo[("epi", r0, 1)]
                h2 = ((x1 - m2) * rstd2) * mod_v[2, 0:1, :] + mod_v[3, 0:1, :]
                h2_v[rs, :] = h2.astype(bf16)
                memo[key] = (toks16(h2),)
            return memo[key][0]

        def params():
            sh = shift_v[...].astype(f32)
            for t in range(4):
                par_v[t] = jnp.broadcast_to(sh[t:t + 1, :], (8, D))
            par_v[4] = jnp.broadcast_to(ssmd_v[...].astype(f32).reshape(1, D), (8, D))

        def mods(lo, hi):
            cc = c_v[...].astype(f32)
            sc = (cc * jax.nn.sigmoid(cc)).astype(bf16)
            sc = jnp.broadcast_to(sc, (16, D))
            md = [jnp.dot(sc, wmod_v[:, i * D:(i + 1) * D], preferred_element_type=f32)[0:8, :] for i in range(lo, hi)]
            return md

        def mods_a():
            sa, ca, ga = mods(0, 3)
            mod_v[0] = ga * (1.0 + ca)
            mod_v[1] = ga * sa

        def mods_b():
            sb, cb = mods(3, 5)
            mod_v[2] = 1.0 + cb
            mod_v[3] = sb

        def mods_c():
            (gb,) = mods(5, 6)
            mod_v[4] = gb

        koff = [0]

        def sel16(tok, base):
            r = jnp.where(never, tok, pltpu.bitcast(base, jnp.int32))
            return pltpu.bitcast(r, bf16)

        def dot_w(lhs, rhs, cells):
            if cells and not (interpret and not force_inj):
                M_, K = lhs.shape
                rowp = []
                for rr in range(M_ // 16):
                    cols_ = []
                    for kt in range(K // 128):
                        base = lhs[rr * 16:(rr + 1) * 16, kt * 128:(kt + 1) * 128]
                        cols_.append(sel16(cells[(rr, kt)](), base) if (rr, kt) in cells else base)
                    rowp.append(jnp.concatenate(cols_, axis=1))
                lhs = jnp.concatenate(rowp, axis=0)
            elif cells:
                for key in sorted(cells):
                    cells[key]()
            return jnp.dot(lhs, rhs, preferred_element_type=f32)

        wait("ft", "shift", "ssmd", ("k", 0), ("v", 0))
        params()
        for r0 in range(0, TM, 16):
            kv_piece(r0)
        wait(("ssmk", 0))
        for b in range(R):
            kspec(b)
            uspec(b)
        wait("g")
        for b in range(R):
            for r in range(T // 8):
                for c in range(5):
                    mac_piece(b, r, c)
            inv(b)
        wait("c", "wmod_a", ("q", 0))
        mods_a()
        for r0 in range(0, TM, 16):
            epi_piece(r0, 1)
        wait("wmod_b")
        mods_b()
        for r0 in range(0, TM, 16):
            epi_piece(r0, 2)

        def out_copy(m):
            return pltpu.make_async_copy(out_v.at[rows(m), :], out_hbm.at[rows(m), :], sems.at[n_in + m])

        GU_T = 5 * TM // 4
        DN_T = (F // 128) * TM // 4
        SP_T = 5 * 256 // 4

        def run_segment(m, ev, streams, paced=None, hold=False):
            avail = [0] * 4
            job = 0
            cells = []
            jobt = {}
            pace_plan = []
            for i, (kind, n, _) in enumerate(ev):
                njob, dur, nrr = {"g": (5, TM, TM // 16), "u": (5, TM, TM // 16), "d": (F // 128, TM, TM // 16),
                                  "ks": (5, 256, 0), "us": (5, 256, 0), "inv": (10, 128, 0), "mc": (25, 16, 0)}[kind]
                for kt in range(njob):
                    t0 = avail[job % 4]
                    jobt[(i, kt)] = t0
                    avail[job % 4] += dur
                    job += 1
                    cells += [(t0 + 16 * rr, i, rr, kt) for rr in range(nrr)]
            cells.sort()
            used = set()
            assign = {i: {} for i in range(len(ev))}

            def getter(memo, th, k_):
                def get():
                    if not memo:
                        memo.append(th())
                    return memo[0][k_]
                return get

            for thunks, ntoks, wts, (ta, tb) in streams:
                inwin = [c_ for c_ in cells if ta <= c_[0] < tb]
                toks = []
                for p_, th in enumerate(thunks):
                    memo_ = []
                    ntok = ntoks[p_] if isinstance(ntoks, list) else ntoks
                    wt = wts[p_] if isinstance(wts, list) else wts
                    toks += [(getter(memo_, th, k_), wt / ntok) for k_ in range(ntok)]
                wsum = sum(w_ for _, w_ in toks)
                acc_ = 0.0
                for get, w_ in toks:
                    acc_ += w_
                    idx = min(len(inwin) - 1, int(acc_ / wsum * len(inwin)))
                    while inwin[idx] in used:
                        idx = (idx - 1) % len(inwin)
                    used.add(inwin[idx])
                    _, i, rr, kt = inwin[idx]
                    assign[i][(rr, kt)] = get
            if paced is not None and do_pace:
                r0s, ta, tb = paced
                pace_plan = [(ta + (tb - ta) * p_ / len(r0s), r0_) for p_, r0_ in enumerate(r0s)]
            for i, (kind, n, _) in enumerate(ev):
                cols = slice(n * NT, (n + 1) * NT)
                if kind == "ks":
                    kspec(n)
                elif kind == "us":
                    uspec(n)
                elif kind == "inv":
                    inv(n)
                elif kind == "mc":
                    mods_c()
                elif kind == "g":
                    gbox[0] = dot_w(h2_v[rows(m), :], wg_v[:, cols], assign[i])
                elif kind == "u":
                    uval = dot_w(h2_v[rows(m), :], wu_v[:, cols], assign[i])
                    hh_v[:, cols] = (gbox[0] * uval).astype(bf16)
                elif kind == "d":
                    p = None
                    for w_ in range(KSP):
                        ks_ = slice(w_ * (F // KSP), (w_ + 1) * (F // KSP))
                        nk_ = F // KSP // 128
                        sub = {(rr, kt - w_ * nk_): g_ for (rr, kt), g_ in assign[i].items() if w_ * nk_ <= kt < (w_ + 1) * nk_}
                        pp = dot_w(hh_v[:, ks_], wd_v[ks_, cols], sub)
                        for (tj, r0_) in list(pace_plan):
                            rr_ = int((tj - jobt[(i, w_ * nk_ + nk_ - 1)]) // 16)
                            if rr_ < TM // 16:
                                pace_plan.remove((tj, r0_))
                                rr_ = max(rr_, 0)
                                pace[r0_] = pp[rr_ * 16:rr_ * 16 + 8, :]
                        p = pp if p is None else p + pp
                    held.append((cols, p))
                    if not hold:
                        for cols_, p_ in held:
                            out_v[rows(m), cols_] = (x1_v[rows(m), cols_] + mod_v[4, 0:1, cols_] * p_).astype(bf16)
                        held.clear()

        gbox = [None]
        held = []

        def gu(ns):
            ev = []
            for n in ns:
                ev += [("g", n, GU_T), ("u", n, GU_T)]
            return ev

        def t_of(ev, kind, last=False):
            tt = 0
            res = None
            for e in ev:
                if e[0] == kind and (res is None or last):
                    res = tt
                tt += e[2]
            return tt if res is None else res

        def kv_stream(mm, win):
            return ([functools.partial(kv_piece, r0) for r0 in range(mm * TM, (mm + 1) * TM, 16)], 5, 1.0, win)

        def mac_stream(mm, win):
            th = []
            for b in range(mm * R, (mm + 1) * R):
                nsub = -(-(b + 1) // tps)
                cuts = [((b + 1) * k_) // nsub for k_ in range(nsub + 1)]
                for r in range(T // 8):
                    for c in range(5):
                        for k_ in range(nsub):
                            th.append(functools.partial(mac_piece, b, r, c, tuple(cuts), k_))
            return (th, 1, 1.0, win)

        def epi_stream(mm, win):
            r0s = list(range(mm * TM, (mm + 1) * TM, 16))
            order = sorted([(p_ + lag * st, st, r0) for p_, r0 in enumerate(r0s) for st in range(3)])
            return ([functools.partial(epi_piece, r0, st) for _, st, r0 in order], [1 if st < 2 else 5 for _, st, r0 in order], [ew[st] for _, st, r0 in order], win)

        def blks(kind, mm):
            return [(kind, b, SP_T) for b in range(mm * R, (mm + 1) * R)]

        pending_out = []
        started = []
        for m in (range(NM) if units is None else units):
            m1, m2 = m + 1, m + 2
            if m == 0:
                for c_ in range(3):
                    wait(("wg", c_), ("wu", c_))
                    run_segment(0, gu(range(WCH[c_], WCH[c_ + 1])), [])
                wait(("k", 1), ("v", 1), ("ssmk", 1))
                for r0 in range(TM, 2 * TM, 16):
                    kv_piece(r0)
                for b in range(R, 2 * R):
                    kspec(b); uspec(b)
                wait(("wg", 3), ("wu", 3))
                ev = gu(range(WCH[3], WCH[4])) + blks("inv", 1)
                run_segment(0, ev, [mac_stream(1, (0, t_of(ev, "inv") - 2 * GU_T))])
                wait(("q", 1), ("wd", 0))
                r0s = list(range(TM, 2 * TM, 16))
                ev = [("d", n, DN_T) for n in range(DCH[0], DCH[1])]
                run_segment(0, ev, [([functools.partial(epi_piece, r0, 1) for r0 in r0s], 1, 1.0, (100, t_of(ev, "x") - t_e[1]))], hold=True)
                wait("wmod_c", ("wd", 1))
                mods_c()
                ev = [("d", n, DN_T) for n in range(DCH[1], DCH[2])]
                run_segment(0, ev, [([functools.partial(epi_piece, r0, 2) for r0 in r0s], 5, 1.0, (0, t_of(ev, "x") - t_e[1]))])
                wait(("wd", 2))
                run_segment(0, [("d", n, DN_T) for n in range(DCH[2], DCH[3])], [])
                continue
            pre = m == 1
            w_kv = w_kv1 * ((1 if m2 < NM else 0) + (1 if pre else 0))
            w_m = 680 * (sum(b + 1 for b in range(m1 * R, (m1 + 1) * R))) if m1 < NM else 0
            w_e = w_e1 if m1 < NM else 0
            t_ffn = 2 * NGU * GU_T + NDN * DN_T
            t_a = t_ffn * w_kv / max(w_kv + w_m + w_e, 1)
            t_b = t_ffn * (w_kv + w_m) / max(w_kv + w_m + w_e, 1)
            ninv = min(NDN - 2, max(0, round((t_b - 2 * NGU * GU_T) / DN_T)))
            n_us = min(NGU - 2, max(1, int((t_a + GU_T) // (2 * GU_T))))
            ev = []
            n0 = 0
            if pre:
                out_copy(0).start(); started.append(0)
                n0 = pre_n0
                run_segment(m, gu(range(n0)), [])
                wait(("k", m1), ("v", m1), ("ssmk", m1))
                ev = blks("ks", m1) + gu(range(n0, n0 + 2)) + blks("us", m1) + gu(range(n0 + 2, n0 + 3))
                run_segment(m, ev, [kv_stream(m1, (0, t_of(ev, "us") - GU_T))])
                n0 += 3
                ev = []
                n_us = min(NGU - 1, n0 + 2)
                ninv = 3
            if m2 < NM:
                ev += blks("ks", m2)
            for n in range(n0, NGU):
                ev += gu([n])
                if n == n_us and m2 < NM:
                    ev += blks("us", m2)
            for n in range(NDN):
                if n == ninv and m1 < NM:
                    ev += blks("inv", m1)
                ev.append(("d", n, DN_T))
            t_end = t_of(ev, "x")
            streams = []
            t0m = t_m[0]
            if m2 < NM:
                t1k = t_of(ev, "us", True) - 2 * SP_T - GU_T
                streams.append(kv_stream(m2, (0, t1k)))
                if not pre:
                    t0m = max(t0m, t1k * mk_ov)
            if m1 < NM:
                t_inv_ = t_of(ev, "inv")
                streams.append(mac_stream(m1, (t0m, t_inv_ - t_m[1])))
                streams.append(epi_stream(m1, (t_inv_ + 2 * SP_T + t_e[0], t_end - t_e[1])))
            if not pre:
                pending_out.append(m - 1)
            if m not in merge:
                for mo in pending_out:
                    out_copy(mo).start(); started.append(mo)
                pending_out.clear()
                hi = m2 + 1 if (m + 1) in merge else m2
                for mm_ in range(m1, min(hi, NM - 1) + 1):
                    wait(("k", mm_), ("v", mm_), ("ssmk", mm_), ("q", mm_))
            paced = None
            if m1 < NM:
                paced = (list(range(m1 * TM, (m1 + 1) * TM, 16)), t_inv_ + 2 * SP_T + pace_w[0], t_end - pace_w[1])
            run_segment(m, ev, streams, paced)
        ms = list(range(NM) if units is None else units)
        for mo in pending_out + [ms[-1]]:
            out_copy(mo).start(); started.append(mo)
        for mo in started:
            out_copy(mo).wait()
        for name, _, _ in plan:
            wait(name)

    def run(A_q, A_k, A_v, A_shift_k, A_ssm_k, A_ssm_D, B_x, B_w_gate, B_w_up, B_w_down, c, w_mod):
        ft, g = _dft_consts()
        any_ = pl.BlockSpec(memory_space=pl.ANY)
        V = pltpu.VMEM
        nsem = 12 + 4 * NM + 2 * NWC + len(DCH) + NM
        out = pl.pallas_call(
            kernel,
            out_shape=jax.ShapeDtypeStruct((S, D), bf16),
            in_specs=[any_] * 13 + [pl.BlockSpec(memory_space=pltpu.SMEM)],
            out_specs=any_,
            scratch_shapes=[
                V((S, D), bf16), V((S, D), bf16), V((S, D), bf16), V((4, D), bf16), V((D, S), bf16), V((D,), bf16),
                V((D, F), bf16), V((D, F), bf16), V((F, D), bf16), V((1, D), bf16), V((D, 6 * D), bf16),
                V((2 * T, T), bf16), V((T, 2 * T), bf16),
                V((2 * NB, 2 * T, D), f32), V((2, 2 * T, D), f32), V((S, D), bf16),
                V((2 * R, 2 * T, D), bf16), V((2 * R, T, D), f32), V((S, D), bf16), V((S, D), f32),
                V((S, D), bf16), V((5, 8, D), f32), V((5, 8, D), f32), V((TM, F), bf16),
                pltpu.SemaphoreType.DMA((nsem,)),
            ],
            compiler_params=pltpu.CompilerParams(vmem_limit_bytes=vmem_mb * 1024 * 1024, flags=flags),
            interpret=interpret,
        )(A_q.reshape(S, D), A_k.reshape(S, D), A_v.reshape(S, D), A_shift_k.T, A_ssm_k, A_ssm_D,
          B_w_gate, B_w_up, B_w_down, c, w_mod, ft, g, np.zeros((1,), np.int32))
        return out.reshape(1, S, D)
    return run


_run = make_kernel()


@jax.jit
def pallas_adaLN_cond__ssm_conv_h3__glu_gated_bilinear__prompt_kernel(
    A_q: jax.Array,
    A_k: jax.Array,
    A_v: jax.Array,
    A_shift_k: jax.Array,
    A_ssm_k: jax.Array,
    A_ssm_D: jax.Array,
    B_x: jax.Array,
    B_w_gate: jax.Array,
    B_w_up: jax.Array,
    B_w_down: jax.Array,
    c: jax.Array,
    w_mod: jax.Array,
):
    return _run(A_q, A_k, A_v, A_shift_k, A_ssm_k, A_ssm_D, B_x, B_w_gate, B_w_up, B_w_down, c, w_mod)
```

```python
import functools
import numpy as np
import jax
import jax.numpy as jnp
from jax import lax
from jax.experimental import pallas as pl
from jax.experimental.pallas import tpu as pltpu

S, D, F = 2048, 640, 1536
T = 128
NB = S // T
H = T // 2
EPS = 1e-5
bf16 = jnp.bfloat16
f32 = jnp.float32


def _dft_consts():
    n = np.arange(T)
    f = np.concatenate([np.arange(0, T, 2), np.arange(1, T, 2)])
    ph = ((2 * f[:, None] + 1) * n[None, :]) % (4 * T)
    ang = 2.0 * np.pi * ph / (4 * T)
    c_, s_ = np.cos(ang).reshape(T // 8, 8, T), -np.sin(ang).reshape(T // 8, 8, T)
    fwd = np.concatenate([c_, s_], axis=1).reshape(2 * T, T)
    inv = fwd.T / T
    return fwd.astype(np.float32).astype(bf16), inv.astype(np.float32).astype(bf16)


def make_kernel(interpret=False, TM=256, WCH=(0, 2, 4, 8, 12), DCH=(0, 2, 5), units=None, vmem_mb=100, flags=None,
                t_kv=(0, 1500), t_us=4, t_m=(0, 500), n_inv=2, t_e=(1, 400), t_ks=-1, nslot_g=60, nslot_d=100, inj='lhs', kstep=2, force_inj=False, skew=False, n_us_s=4, pw=(300, 1200, 6000), n_e0=7, dynz=False, etok=True, pre_n0=2, dbg_waitall=False, merge=(), KSP=3, do_pace=True, pace_w=(200, 1200), yval=True, ew=(60., 150., 70.), w_kv1=3500, w_e1=7000, mk_ov=1.0, tps=5, lag=2, bsel=True, scopes=False):
    R = TM // T
    NM = S // TM
    NT = 128
    NGU = F // NT
    NDN = D // NT
    NWC = len(WCH) - 1

    def kernel(q_hbm, k_hbm, v_hbm, shift_hbm, ssmk_hbm, ssmd_hbm, wg_hbm, wu_hbm, wd_hbm, c_hbm, wmod_hbm,
               ft_hbm, g_hbm, zero_smem, out_hbm,
               q_v, k_v, v_v, shift_v, ssmk_v, ssmd_v, wg_v, wu_v, wd_v, c_v, wmod_v, ft_v, g_v,
               sp_v, kraw_v, kv_v, z_v, y_v, h2_v, x1_v, out_v, mod_v, par_v, hh_v, p0_v, sems):
        never = zero_smem[0] > 0

        plan = []

        def add(name, src, dst):
            plan.append((name, src, dst))

        def rows(m):
            return slice(m * TM, (m + 1) * TM)

        def add_kv(m):
            add(("k", m), k_hbm.at[rows(m)], k_v.at[rows(m)])
            add(("v", m), v_hbm.at[rows(m)], v_v.at[rows(m)])

        def add_s(m):
            add(("ssmk", m), ssmk_hbm.at[:, rows(m)], ssmk_v.at[:, rows(m)])

        def add_q(m):
            add(("q", m), q_hbm.at[rows(m)], q_v.at[rows(m)])

        def add_w(c):
            cols = slice(WCH[c] * NT, WCH[c + 1] * NT)
            add(("wg", c), wg_hbm.at[:, cols], wg_v.at[:, cols])
            add(("wu", c), wu_hbm.at[:, cols], wu_v.at[:, cols])

        def add_wd(c):
            cols = slice(DCH[c] * NT, DCH[c + 1] * NT)
            add(("wd", c), wd_hbm.at[:, cols], wd_v.at[:, cols])

        add("ft", ft_hbm, ft_v)
        add("shift", shift_hbm, shift_v)
        add("ssmd", ssmd_hbm, ssmd_v)
        add_kv(0); add_s(0)
        add("g", g_hbm, g_v)
        add_kv(1); add_s(1)
        add("c", c_hbm, c_v)
        add("wmod_a", wmod_hbm.at[:, 0:3 * D], wmod_v.at[:, 0:3 * D])
        add_q(0); add_q(1)
        add("wmod_b", wmod_hbm.at[:, 3 * D:5 * D], wmod_v.at[:, 3 * D:5 * D])
        for c_ in range(NWC):
            add_w(c_)
        add_kv(2); add_s(2)
        add_wd(0); add_wd(1)
        add_kv(3); add_s(3)
        add("wmod_c", wmod_hbm.at[:, 5 * D:6 * D], wmod_v.at[:, 5 * D:6 * D])
        add_q(2); add_q(3)
        for m in range(4, NM):
            add_kv(m); add_s(m); add_q(m)
        cps = {}
        for i, (name, src, dst) in enumerate(plan):
            cps[name] = pltpu.make_async_copy(src, dst, sems.at[i])
        n_in = len(plan)
        for name, _, _ in plan:
            cps[name].start()
        waited = set()

        def wait(*names):
            for name in names:
                if name not in waited:
                    waited.add(name)
                    if scopes:
                        with jax.named_scope("w_" + "_".join(map(str, name)) if isinstance(name, tuple) else "w_" + name):
                            cps[name].wait()
                    else:
                        cps[name].wait()

        if dbg_waitall:
            for name, _, _ in plan:
                wait(name)
            units_ = []
        def i32(x):
            return pltpu.bitcast(x, jnp.int32)

        def toks16(x):
            xi = i32(x[0:8]) ^ i32(x[8:16])
            return [xi[:, c * 128:(c + 1) * 128] for c in range(5)]

        def kspec(d):
            kblk = ssmk_v[:, d * T:(d + 1) * T]
            raw = lax.dot_general(ft_v[...], kblk, (((1,), (1,)), ((), ())), preferred_element_type=f32)
            if d == 0:
                sp_v[NB] = raw
            else:
                p = (d - 1) % 2
                for g in range(T // 8):
                    re = slice(16 * g, 16 * g + 8)
                    im = slice(16 * g + 8, 16 * g + 16)
                    if g < T // 16:
                        sp_v[NB + d, re, :] = raw[re] - kraw_v[p, im, :]
                        sp_v[NB + d, im, :] = raw[im] + kraw_v[p, re, :]
                    else:
                        sp_v[NB + d, re, :] = raw[re] + kraw_v[p, im, :]
                        sp_v[NB + d, im, :] = raw[im] - kraw_v[p, re, :]
            if d < NB - 1:
                kraw_v[d % 2] = raw

        def uspec(j):
            sp_v[j] = jnp.dot(ft_v[...], kv_v[j * T:(j + 1) * T, :], preferred_element_type=f32)

        def kv_piece(r0):
            kc = k_v[r0:r0 + 16, :].astype(f32)
            if r0 == 0:
                kp = jnp.zeros((8, D), f32)
            else:
                kp = k_v[r0 - 16:r0, :].astype(f32)[8:16]
            ext = jnp.concatenate([kp, kc], axis=0)
            ks = kc * par_v[0, 0:1, :]
            for t in range(1, 4):
                ks = ks + ext[8 - t:24 - t] * par_v[t, 0:1, :]
            kvf = ks * v_v[r0:r0 + 16, :].astype(f32)
            kv_v[r0:r0 + 16, :] = kvf.astype(bf16)
            return toks16(kvf)

        memo = {}
        zoff = [0]
        pace = {}

        def mac_piece(i, r, c, cuts=None, k_=None):
            if cuts is None:
                cuts, k_ = (0, i + 1), 0
            key = ("mac", i, r, c, k_)
            if key in memo:
                return memo[key][2]
            zb = i % (2 * R)
            re = slice(r * 16, r * 16 + 8)
            im = slice(r * 16 + 8, r * 16 + 16)
            cs = slice(c * 128, (c + 1) * 128)
            ar = ai = None
            if k_ > 0:
                mac_piece(i, r, c, cuts, k_ - 1)
                ar, ai, _ = memo[("mac", i, r, c, k_ - 1)]
            for j in range(cuts[k_], cuts[k_ + 1]):
                kr = sp_v[zoff[0] + (NB + i - j), re, cs]
                ki = sp_v[zoff[0] + (NB + i - j), im, cs]
                ur = sp_v[zoff[0] + j, re, cs]
                ui = sp_v[zoff[0] + j, im, cs]
                tr = kr * ur - ki * ui
                ti = kr * ui + ki * ur
                ar = tr if ar is None else ar + tr
                ai = ti if ai is None else ai + ti
            if cuts[k_ + 1] == i + 1:
                z_v[zb, r * 16:r * 16 + 16, cs] = jnp.concatenate([ar, ai], axis=0).astype(bf16)
            memo[key] = (ar, ai, [i32(ar) ^ i32(ai)])
            return memo[key][2]

        def inv(i):
            yv = jnp.dot(g_v[...], z_v[i % (2 * R)], preferred_element_type=f32)
            if yval:
                memo[("y", i)] = yv
            else:
                y_v[i % (2 * R)] = yv

        def moments(x):
            m = jnp.sum(x, axis=-1, keepdims=True) * (1.0 / D)
            q = jnp.sum(x * x, axis=-1, keepdims=True) * (1.0 / D)
            rstd = lax.rsqrt(jnp.maximum(q - m * m, 0.0) + EPS)
            return m, rstd

        def btok(v):
            vb = jnp.broadcast_to(v, (16, 128))
            return i32(vb[0:8]) ^ i32(vb[8:16])

        def epi_piece(r0, stage=2):
            key = ("epi", r0, stage)
            if key in memo:
                return memo[key][0]
            i = r0 // T
            rs = slice(r0, r0 + 16)
            if stage == 0:
                x = q_v[rs, :].astype(f32)
                if r0 in pace:
                    x = jnp.where(never, jnp.tile(pace.pop(r0), (2, 5)), x)
                m, rstd = moments(x)
                memo[key] = ([btok(rstd) ^ btok(m)], m, rstd, x)
            elif stage == 1:
                epi_piece(r0, 0)
                _, m, rstd, x = memo[("epi", r0, 0)]
                if yval:
                    yc = memo[("y", i)][r0 - i * T:r0 - i * T + 16]
                else:
                    yc = y_v[i % (2 * R), r0 - i * T:r0 - i * T + 16, :]
                y = yc + kv_v[rs, :].astype(f32) * par_v[4, 0:1, :]
                x1 = x + (((x - m) * rstd) * mod_v[0, 0:1, :] + mod_v[1, 0:1, :]) * y
                x1_v[rs, :] = x1
                m2, rstd2 = moments(x1)
                memo[key] = ([btok(rstd2) ^ btok(m2)], x1, m2, rstd2)
            else:
                epi_piece(r0, 1)
                _, x1, m2, rstd2 = memo[("epi", r0, 1)]
                h2 = ((x1 - m2) * rstd2) * mod_v[2, 0:1, :] + mod_v[3, 0:1, :]
                h2_v[rs, :] = h2.astype(bf16)
                memo[key] = (toks16(h2),)
            return memo[key][0]

        def fin_piece(r0):
            rs = slice(r0, r0 + 16)
            o = x1_v[rs, :] + mod_v[4, 0:1, :] * p0_v[rs, :]
            out_v[rs, :] = o.astype(bf16)
            return toks16(o)

        def params():
            sh = shift_v[...].astype(f32)
            for t in range(4):
                par_v[t] = jnp.broadcast_to(sh[t:t + 1, :], (8, D))
            par_v[4] = jnp.broadcast_to(ssmd_v[...].astype(f32).reshape(1, D), (8, D))

        def mods(lo, hi):
            cc = c_v[...].astype(f32)
            sc = (cc * jax.nn.sigmoid(cc)).astype(bf16)
            sc = jnp.broadcast_to(sc, (16, D))
            md = [jnp.dot(sc, wmod_v[:, i * D:(i + 1) * D], preferred_element_type=f32)[0:8, :] for i in range(lo, hi)]
            return md

        def mods_a():
            sa, ca, ga = mods(0, 3)
            mod_v[0] = ga * (1.0 + ca)
            mod_v[1] = ga * sa

        def mods_b():
            sb, cb = mods(3, 5)
            mod_v[2] = 1.0 + cb
            mod_v[3] = sb

        def mods_c():
            (gb,) = mods(5, 6)
            mod_v[4] = gb

        koff = [0]

        def sel16(tok, base):
            r = jnp.where(never, tok, pltpu.bitcast(base, jnp.int32))
            return pltpu.bitcast(r, bf16)

        def dot_w(lhs, rhs, cells):
            if cells and not (interpret and not force_inj):
                M_, K = lhs.shape
                rowp = []
                for rr in range(M_ // 16):
                    cols_ = []
                    for kt in range(K // 128):
                        base = lhs[rr * 16:(rr + 1) * 16, kt * 128:(kt + 1) * 128]
                        cols_.append(sel16(cells[(rr, kt)](), base) if (rr, kt) in cells else base)
                    rowp.append(jnp.concatenate(cols_, axis=1))
                lhs = jnp.concatenate(rowp, axis=0)
            elif cells:
                for key in sorted(cells):
                    cells[key]()
            return jnp.dot(lhs, rhs, preferred_element_type=f32)

        wait("ft", "shift", "ssmd", ("k", 0), ("v", 0))
        params()
        for u_ in range(2):
            wait(("k", u_), ("v", u_))
            for r0 in range(u_ * TM, (u_ + 1) * TM, 16):
                kv_piece(r0)
            wait(("ssmk", u_))
            for b in range(u_ * R, (u_ + 1) * R):
                kspec(b)
                uspec(b)
            wait("g")
            for b in range(u_ * R, (u_ + 1) * R):
                for r in range(T // 8):
                    for c in range(5):
                        mac_piece(b, r, c)
                inv(b)
        wait("c", "wmod_a", ("q", 0), ("q", 1))
        mods_a()
        for r0 in range(0, 2 * TM, 16):
            epi_piece(r0, 1)
        wait("wmod_b")
        mods_b()
        for r0 in range(0, 2 * TM, 16):
            epi_piece(r0, 2)

        def out_copy(m):
            return pltpu.make_async_copy(out_v.at[rows(m), :], out_hbm.at[rows(m), :], sems.at[n_in + m])

        GU_T = 5 * TM // 4
        DN_T = (F // 128) * TM // 4
        SP_T = 5 * 256 // 4

        def run_segment(m, ev, streams, paced=None, hold=False):
            avail = [0] * 4
            job = 0
            cells = []
            jobt = {}
            pace_plan = []
            for i, (kind, n, _) in enumerate(ev):
                njob, dur, nrr = {"g": (5, TM, TM // 16), "u": (5, TM, TM // 16), "d": (F // 128, TM, TM // 16),
                                  "ks": (5, 256, 0), "us": (5, 256, 0), "inv": (10, 128, 0), "mc": (25, 16, 0)}[kind]
                for kt in range(njob):
                    t0 = avail[job % 4]
                    jobt[(i, kt)] = t0
                    avail[job % 4] += dur
                    job += 1
                    cells += [(t0 + 16 * rr, i, rr, kt) for rr in range(nrr)]
            cells.sort()
            used = set()
            assign = {i: {} for i in range(len(ev))}

            def getter(memo, th, k_):
                def get():
                    if not memo:
                        memo.append(th())
                    return memo[0][k_]
                return get

            for thunks, ntoks, wts, (ta, tb) in streams:
                inwin = [c_ for c_ in cells if ta <= c_[0] < tb]
                toks = []
                for p_, th in enumerate(thunks):
                    memo_ = []
                    ntok = ntoks[p_] if isinstance(ntoks, list) else ntoks
                    wt = wts[p_] if isinstance(wts, list) else wts
                    toks += [(getter(memo_, th, k_), wt / ntok) for k_ in range(ntok)]
                wsum = sum(w_ for _, w_ in toks)
                acc_ = 0.0
                for get, w_ in toks:
                    acc_ += w_
                    idx = min(len(inwin) - 1, int(acc_ / wsum * len(inwin)))
                    while inwin[idx] in used:
                        idx = (idx - 1) % len(inwin)
                    used.add(inwin[idx])
                    _, i, rr, kt = inwin[idx]
                    assign[i][(rr, kt)] = get
            if paced is not None and do_pace:
                r0s, ta, tb = paced
                pace_plan = [(ta + (tb - ta) * p_ / len(r0s), r0_) for p_, r0_ in enumerate(r0s)]
            def do_paced(i, last_job, val):
                for (tj, r0_) in list(pace_plan):
                    rr_ = int((tj - jobt[(i, last_job)]) // 16)
                    if rr_ < TM // 16:
                        pace_plan.remove((tj, r0_))
                        rr_ = max(rr_, 0)
                        pace[r0_] = val[rr_ * 16:rr_ * 16 + 8, :]
                        if not etok or skew:
                            epi_piece(r0_, 2)

            for i, (kind, n, _) in enumerate(ev):
                cols = slice(n * NT, (n + 1) * NT)
                if kind == "ks":
                    kspec(n)
                elif kind == "us":
                    uspec(n)
                elif kind == "inv":
                    inv(n)
                elif kind == "mc":
                    mods_c()
                elif kind == "g":
                    gbox[0] = dot_w(h2_v[rows(m), :], wg_v[:, cols], assign[i])
                    do_paced(i, 4, gbox[0])
                elif kind == "u":
                    uval = dot_w(h2_v[rows(m), :], wu_v[:, cols], assign[i])
                    do_paced(i, 4, uval)
                    hh_v[:, cols] = (gbox[0] * uval).astype(bf16)
                elif kind == "d":
                    p = None
                    for w_ in range(KSP):
                        ks_ = slice(w_ * (F // KSP), (w_ + 1) * (F // KSP))
                        nk_ = F // KSP // 128
                        sub = {(rr, kt - w_ * nk_): g_ for (rr, kt), g_ in assign[i].items() if w_ * nk_ <= kt < (w_ + 1) * nk_}
                        pp = dot_w(hh_v[:, ks_], wd_v[ks_, cols], sub)
                        do_paced(i, w_ * nk_ + nk_ - 1, pp)
                        p = pp if p is None else p + pp
                    if hold:
                        p0_v[:, cols] = p
                    else:
                        out_v[rows(m), cols] = (x1_v[rows(m), cols] + mod_v[4, 0:1, cols] * p).astype(bf16)

        gbox = [None]
        held = []

        def gu(ns):
            ev = []
            for n in ns:
                ev += [("g", n, GU_T), ("u", n, GU_T)]
            return ev

        def t_of(ev, kind, last=False):
            tt = 0
            res = None
            for e in ev:
                if e[0] == kind and (res is None or last):
                    res = tt
                tt += e[2]
            return tt if res is None else res

        def kv_stream(mm, win):
            return ([functools.partial(kv_piece, r0) for r0 in range(mm * TM, (mm + 1) * TM, 16)], 5, 1.0, win)

        def mac_stream(mm, win):
            th = []
            for b in range(mm * R, (mm + 1) * R):
                nsub = -(-(b + 1) // tps)
                cuts = [((b + 1) * k_) // nsub for k_ in range(nsub + 1)]
                for r in range(T // 8):
                    for c in range(5):
                        for k_ in range(nsub):
                            th.append(functools.partial(mac_piece, b, r, c, tuple(cuts), k_))
            return (th, 1, 1.0, win)

        def epi_stream(mm, win):
            r0s = list(range(mm * TM, (mm + 1) * TM, 16))
            order = sorted([(p_ + lag * st, st, r0) for p_, r0 in enumerate(r0s) for st in range(3)])
            return ([functools.partial(epi_piece, r0, st) for _, st, r0 in order], [1 if st < 2 else 5 for _, st, r0 in order], [ew[st] for _, st, r0 in order], win)

        def blks(kind, mm):
            return [(kind, b, SP_T) for b in range(mm * R, (mm + 1) * R)]

        pending_out = []
        started = []
        for m in (range(NM) if units is None else units):
            m1, m2 = m + 1, m + 2
            if dynz:
                zoff[0] = zero_smem[m]
            if m == 0:
                for c_ in range(NWC):
                    wait(("wg", c_), ("wu", c_))
                    run_segment(0, gu(range(WCH[c_], WCH[c_ + 1])), [])
                wait(("k", 2), ("v", 2), ("ssmk", 2))
                for r0 in range(2 * TM, 3 * TM, 16):
                    kv_piece(r0)
                for b in range(2 * R, 3 * R):
                    kspec(b); uspec(b)
                for c_ in range(2):
                    wait(("wd", c_))
                    run_segment(0, [("d", n, DN_T) for n in range(DCH[c_], DCH[c_ + 1])], [], hold=True)
                continue
            if skew:
                r1 = list(range(m1 * TM, (m1 + 1) * TM, 16))
                ev = []
                streams = []
                n0 = 0
                if m == 1:
                    run_segment(m, gu(range(pre_n0)), [])
                    wait(("k", m1), ("v", m1), ("ssmk", m1))
                    ev = blks("ks", m1) + gu(range(pre_n0, pre_n0 + 2)) + blks("us", m1) + gu(range(pre_n0 + 2, pre_n0 + 3))
                    run_segment(m, ev, [kv_stream(m1, (0, t_of(ev, "us") - GU_T))])
                    n0 = pre_n0 + 3
                    wait("wmod_c", ("q", m1), ("k", m2), ("v", m2), ("ssmk", m2))
                    pending_out.append(0)
                    ev = [("mc", 0, 100)] + blks("ks", m2) + gu(range(n0, n0 + 3)) + blks("us", m2) + blks("inv", m1) + gu(range(n0 + 3, NGU))
                    ev += [("d", n, DN_T) for n in range(NDN)]
                    tu = t_of(ev, "us")
                    streams.append(kv_stream(m2, (0, tu - GU_T)))
                    streams.append(mac_stream(m1, (0, tu - GU_T)))
                    streams.append(mac_stream(m2, (tu + 4 * SP_T, t_of(ev, "x") - t_m[1])))
                    streams.append(([functools.partial(fin_piece, r0) for r0 in range(0, TM, 16)], 5, 1.0, (t_of(ev, "d"), t_of(ev, "x") - 300)))
                    paced = (r1, tu + 4 * SP_T + 300, t_of(ev, "x") - pw[1])
                    run_segment(m, ev, streams, paced)
                    continue
                out_copy_list = pending_out + [m - 1]
                for mo in out_copy_list:
                    out_copy(mo).start(); started.append(mo)
                pending_out.clear()
                if m1 < NM:
                    wait(("q", m1))
                    ev += blks("inv", m1)
                if m2 < NM:
                    wait(("k", m2), ("v", m2), ("ssmk", m2))
                    ev += blks("ks", m2)
                for n in range(NGU):
                    ev += gu([n])
                    if n == n_us_s and m2 < NM:
                        ev += blks("us", m2)
                ev += [("d", n, DN_T) for n in range(NDN)]
                paced = None
                if m2 < NM:
                    tu = t_of(ev, "us")
                    streams.append(kv_stream(m2, (0, tu - GU_T)))
                    streams.append(mac_stream(m2, (tu + 2 * SP_T + 200, t_of(ev, "x") - t_m[1])))
                if m1 < NM:
                    paced = (r1, t_of(ev, "g") + pw[0], min(t_of(ev, "g") + pw[2], t_of(ev, "x") - pw[1]))
                run_segment(m, ev, streams, paced)
                continue
            pre = False
            first = m == 1
            w_kv = w_kv1 * ((1 if m2 < NM else 0) + (1 if pre else 0))
            w_m = 680 * (sum(b + 1 for b in range(m1 * R, (m1 + 1) * R))) if m1 < NM else 0
            w_e = w_e1 if m1 < NM else 0
            t_ffn = 2 * NGU * GU_T + NDN * DN_T
            t_a = t_ffn * w_kv / max(w_kv + w_m + w_e, 1)
            t_b = t_ffn * (w_kv + w_m) / max(w_kv + w_m + w_e, 1)
            ninv = min(NDN - 2, max(0, round((t_b - 2 * NGU * GU_T) / DN_T)))
            if first:
                ninv = 0
            n_us = min(NGU - 2, max(1, int((t_a + GU_T) // (2 * GU_T))))
            ev = []
            n0 = 0
            if pre:
                n0 = pre_n0
                run_segment(m, gu(range(n0)), [])
                wait(("k", m1), ("v", m1), ("ssmk", m1))
                ev = blks("ks", m1) + gu(range(n0, n0 + 2)) + blks("us", m1) + gu(range(n0 + 2, n0 + 3))
                run_segment(m, ev, [kv_stream(m1, (0, t_of(ev, "us") - GU_T))])
                n0 += 3
                wait("wmod_c")
                pending_out.append(0)
                ev = [("mc", 0, 100)]
                n_us = min(NGU - 1, n0 + 2)
                ninv = 3
            if first:
                ev += [("mc", 0, 100)]
            if m2 < NM:
                ev += blks("ks", m2)
            for n in range(n0, NGU):
                ev += gu([n])
                if n == n_us and m2 < NM:
                    ev += blks("us", m2)
            for n in range(NDN):
                if n == ninv and m1 < NM:
                    ev += blks("inv", m1)
                ev.append(("d", n, DN_T))
            t_end = t_of(ev, "x")
            streams = []
            t0m = t_m[0]
            if m2 < NM:
                t1k = t_of(ev, "us", True) - 2 * SP_T - GU_T
                streams.append(kv_stream(m2, (0, t1k)))
                if not pre:
                    t0m = max(t0m, t1k * mk_ov)
            if first:
                streams.append(([functools.partial(fin_piece, r0) for r0 in range(0, TM, 16)], 5, 1.0, (t_of(ev, "us", True) + 2 * SP_T, t_of(ev, "inv"))))
            if m1 < NM:
                t_inv_ = t_of(ev, "inv")
                streams.append(mac_stream(m1, (t0m, t_inv_ - t_m[1])))
                if etok:
                    streams.append(epi_stream(m1, (t_inv_ + 2 * SP_T + t_e[0], t_end - t_e[1])))
            pending_out.append(m - 1)
            if first:
                wait(("k", m2), ("v", m2), ("ssmk", m2))
                cut = [i for i, e in enumerate(ev) if e[0] in ("d", "inv")][0]
                evA, evB = [e for e in ev[:cut] if e[0] != "mc"], [("mc", 0, 100)] + ev[cut:]
                tA = t_of(evA, "x")
                run_segment(m, evA, [kv_stream(m2, (0, t_of(evA, "us", True) - 2 * SP_T - GU_T)),
                                     mac_stream(m1, (t_of(evA, "us"), tA - t_m[1]))])
                wait("wmod_c", ("q", m1))
                ti = t_of(evB, "inv")
                pending_out.clear(); pending_out.append(0)
                run_segment(m, evB, [([functools.partial(fin_piece, r0) for r0 in range(0, TM, 16)], 5, 1.0, (200, t_of(evB, "x") - 300)),
                                     epi_stream(m1, (ti + 2 * SP_T + t_e[0], t_of(evB, "x") - t_e[1]))],
                            (list(range(m1 * TM, (m1 + 1) * TM, 16)), ti + 2 * SP_T + pace_w[0], t_of(evB, "x") - pace_w[1]))
                continue
            for mo in pending_out:
                out_copy(mo).start(); started.append(mo)
            pending_out.clear()
            for mm_ in range(m1, min(m2, NM - 1) + 1):
                wait(("k", mm_), ("v", mm_), ("ssmk", mm_), ("q", mm_))
            paced = None
            if m1 < NM:
                paced = (list(range(m1 * TM, (m1 + 1) * TM, 16)), t_inv_ + 2 * SP_T + pace_w[0], t_end - pace_w[1])
            run_segment(m, ev, streams, paced)
        ms = list(range(NM) if units is None else units)
        for mo in pending_out + [ms[-1]]:
            out_copy(mo).start(); started.append(mo)
        for mo in started:
            out_copy(mo).wait()
        for name, _, _ in plan:
            wait(name)

    def run(A_q, A_k, A_v, A_shift_k, A_ssm_k, A_ssm_D, B_x, B_w_gate, B_w_up, B_w_down, c, w_mod):
        ft, g = _dft_consts()
        any_ = pl.BlockSpec(memory_space=pl.ANY)
        V = pltpu.VMEM
        nsem = 12 + 4 * NM + 2 * NWC + len(DCH) + NM
        out = pl.pallas_call(
            kernel,
            out_shape=jax.ShapeDtypeStruct((S, D), bf16),
            in_specs=[any_] * 13 + [pl.BlockSpec(memory_space=pltpu.SMEM)],
            out_specs=any_,
            scratch_shapes=[
                V((S, D), bf16), V((S, D), bf16), V((S, D), bf16), V((4, D), bf16), V((D, S), bf16), V((D,), bf16),
                V((D, F), bf16), V((D, F), bf16), V((F, D), bf16), V((1, D), bf16), V((D, 6 * D), bf16),
                V((2 * T, T), bf16), V((T, 2 * T), bf16),
                V((2 * NB, 2 * T, D), f32), V((2, 2 * T, D), f32), V((S, D), bf16),
                V((2 * R, 2 * T, D), bf16), V((2 * R, T, D), f32), V((S, D), bf16), V((S, D), f32),
                V((S, D), bf16), V((5, 8, D), f32), V((5, 8, D), f32), V((TM, F), bf16), V((TM, D), f32),
                pltpu.SemaphoreType.DMA((nsem,)),
            ],
            compiler_params=pltpu.CompilerParams(vmem_limit_bytes=vmem_mb * 1024 * 1024, flags=flags),
            interpret=interpret,
        )(A_q.reshape(S, D), A_k.reshape(S, D), A_v.reshape(S, D), A_shift_k.T, A_ssm_k, A_ssm_D,
          B_w_gate, B_w_up, B_w_down, c, w_mod, ft, g, np.zeros((1,), np.int32))
        return out.reshape(1, S, D)
    return run


_run = make_kernel()


@jax.jit
def pallas_adaLN_cond__ssm_conv_h3__glu_gated_bilinear__prompt_kernel(
    A_q: jax.Array,
    A_k: jax.Array,
    A_v: jax.Array,
    A_shift_k: jax.Array,
    A_ssm_k: jax.Array,
    A_ssm_D: jax.Array,
    B_x: jax.Array,
    B_w_gate: jax.Array,
    B_w_up: jax.Array,
    B_w_down: jax.Array,
    c: jax.Array,
    w_mod: jax.Array,
):
    return _run(A_q, A_k, A_v, A_shift_k, A_ssm_k, A_ssm_D, B_x, B_w_gate, B_w_up, B_w_down, c, w_mod)
```

```python
import functools
import numpy as np
import jax
import jax.numpy as jnp
from jax import lax
from jax.experimental import pallas as pl
from jax.experimental.pallas import tpu as pltpu

S, D, F = 2048, 640, 1536
T = 128
NB = S // T
H = T // 2
EPS = 1e-5
bf16 = jnp.bfloat16
f32 = jnp.float32


def _dft_consts():
    n = np.arange(T)
    f = np.concatenate([np.arange(0, T, 2), np.arange(1, T, 2)])
    ph = ((2 * f[:, None] + 1) * n[None, :]) % (4 * T)
    ang = 2.0 * np.pi * ph / (4 * T)
    c_, s_ = np.cos(ang).reshape(T // 8, 8, T), -np.sin(ang).reshape(T // 8, 8, T)
    fwd = np.concatenate([c_, s_], axis=1).reshape(2 * T, T)
    inv = fwd.T / T
    return fwd.astype(np.float32).astype(bf16), inv.astype(np.float32).astype(bf16)


def make_kernel(interpret=False, scopes=False, force_inj=False, units=None, vmem_mb=100, flags=None):
    TM = 256
    WCH = (0, 2, 4, 6, 8, 10, 12)
    DCH = (0, 2, 5)
    t_m, t_e, pace_w, ew = (0, 500), (1, 400), (200, 1200), (60., 150., 70.)
    w_kv1, w_e1, mk_ov, tps, lag, KSP, tail_split = 3500, 7000, 1.0, 6, 2, 3, 4
    etok = do_pace = yval = True
    R = TM // T
    NM = S // TM
    NT = 128
    NGU = F // NT
    NDN = D // NT
    NWC = len(WCH) - 1

    def kernel(q_hbm, k_hbm, v_hbm, shift_hbm, ssmk_hbm, ssmd_hbm, wg_hbm, wu_hbm, wd_hbm, c_hbm, wmod_hbm,
               ft_hbm, g_hbm, zero_smem, out_hbm,
               q_v, k_v, v_v, shift_v, ssmk_v, ssmd_v, wg_v, wu_v, wd_v, c_v, wmod_v, ft_v, g_v,
               sp_v, kraw_v, kv_v, z_v, y_v, h2_v, x1_v, out_v, mod_v, par_v, hh_v, p0_v, sems):
        never = zero_smem[0] > 0

        plan = []

        def add(name, src, dst):
            plan.append((name, src, dst))

        def rows(m):
            return slice(m * TM, (m + 1) * TM)

        def add_kv(m):
            add(("k", m), k_hbm.at[rows(m)], k_v.at[rows(m)])
            add(("v", m), v_hbm.at[rows(m)], v_v.at[rows(m)])

        def add_s(m):
            add(("ssmk", m), ssmk_hbm.at[:, rows(m)], ssmk_v.at[:, rows(m)])

        def add_q(m):
            add(("q", m), q_hbm.at[rows(m)], q_v.at[rows(m)])

        def add_w(c):
            cols = slice(WCH[c] * NT, WCH[c + 1] * NT)
            add(("wg", c), wg_hbm.at[:, cols], wg_v.at[:, cols])
            add(("wu", c), wu_hbm.at[:, cols], wu_v.at[:, cols])

        def add_wd(c):
            cols = slice(DCH[c] * NT, DCH[c + 1] * NT)
            add(("wd", c), wd_hbm.at[:, cols], wd_v.at[:, cols])

        add("ft", ft_hbm, ft_v)
        add("shift", shift_hbm, shift_v)
        add("ssmd", ssmd_hbm, ssmd_v)
        add_kv(0); add_s(0)
        add("g", g_hbm, g_v)
        add_kv(1); add_s(1)
        add("c", c_hbm, c_v)
        add("wmod_a", wmod_hbm.at[:, 0:3 * D], wmod_v.at[:, 0:3 * D])
        add_q(0); add_q(1)
        add("wmod_b", wmod_hbm.at[:, 3 * D:5 * D], wmod_v.at[:, 3 * D:5 * D])
        for c_ in range(NWC):
            add_w(c_)
        add_kv(2); add_s(2)
        add_wd(0); add_wd(1)
        add_kv(3); add_s(3)
        add("wmod_c", wmod_hbm.at[:, 5 * D:6 * D], wmod_v.at[:, 5 * D:6 * D])
        add_q(2); add_q(3)
        for m in range(4, NM):
            add_kv(m); add_s(m); add_q(m)
        cps = {}
        for i, (name, src, dst) in enumerate(plan):
            cps[name] = pltpu.make_async_copy(src, dst, sems.at[i])
        n_in = len(plan)
        for name, _, _ in plan:
            cps[name].start()
        waited = set()

        def wait(*names):
            for name in names:
                if name not in waited:
                    waited.add(name)
                    if scopes:
                        with jax.named_scope("w_" + "_".join(map(str, name)) if isinstance(name, tuple) else "w_" + name):
                            cps[name].wait()
                    else:
                        cps[name].wait()

        def i32(x):
            return pltpu.bitcast(x, jnp.int32)

        def toks16(x):
            xi = i32(x[0:8]) ^ i32(x[8:16])
            return [xi[:, c * 128:(c + 1) * 128] for c in range(5)]

        def kspec(d):
            kblk = ssmk_v[:, d * T:(d + 1) * T]
            raw = lax.dot_general(ft_v[...], kblk, (((1,), (1,)), ((), ())), preferred_element_type=f32)
            if d == 0:
                sp_v[NB] = raw
            else:
                p = (d - 1) % 2
                for g in range(T // 8):
                    re = slice(16 * g, 16 * g + 8)
                    im = slice(16 * g + 8, 16 * g + 16)
                    if g < T // 16:
                        sp_v[NB + d, re, :] = raw[re] - kraw_v[p, im, :]
                        sp_v[NB + d, im, :] = raw[im] + kraw_v[p, re, :]
                    else:
                        sp_v[NB + d, re, :] = raw[re] + kraw_v[p, im, :]
                        sp_v[NB + d, im, :] = raw[im] - kraw_v[p, re, :]
            if d < NB - 1:
                kraw_v[d % 2] = raw

        def uspec(j):
            sp_v[j] = jnp.dot(ft_v[...], kv_v[j * T:(j + 1) * T, :], preferred_element_type=f32)

        def kv_piece(r0):
            kc = k_v[r0:r0 + 16, :].astype(f32)
            if r0 == 0:
                kp = jnp.zeros((8, D), f32)
            else:
                kp = k_v[r0 - 16:r0, :].astype(f32)[8:16]
            ext = jnp.concatenate([kp, kc], axis=0)
            ks = kc * par_v[0, 0:1, :]
            for t in range(1, 4):
                ks = ks + ext[8 - t:24 - t] * par_v[t, 0:1, :]
            kvf = ks * v_v[r0:r0 + 16, :].astype(f32)
            kv_v[r0:r0 + 16, :] = kvf.astype(bf16)
            return toks16(kvf)

        memo = {}

        pace = {}

        def mac_piece(i, r, c, cuts=None, k_=None):
            if cuts is None:
                cuts, k_ = (0, i + 1), 0
            key = ("mac", i, r, c, k_)
            if key in memo:
                return memo[key][2]
            zb = i % (2 * R)
            re = slice(r * 16, r * 16 + 8)
            im = slice(r * 16 + 8, r * 16 + 16)
            cs = slice(c * 128, (c + 1) * 128)
            ar = ai = None
            if k_ > 0:
                mac_piece(i, r, c, cuts, k_ - 1)
                ar, ai, _ = memo[("mac", i, r, c, k_ - 1)]
            for j in range(cuts[k_], cuts[k_ + 1]):
                kr = sp_v[NB + i - j, re, cs]
                ki = sp_v[NB + i - j, im, cs]
                ur = sp_v[j, re, cs]
                ui = sp_v[j, im, cs]
                tr = kr * ur - ki * ui
                ti = kr * ui + ki * ur
                ar = tr if ar is None else ar + tr
                ai = ti if ai is None else ai + ti
            if cuts[k_ + 1] == i + 1:
                z_v[zb, r * 16:r * 16 + 16, cs] = jnp.concatenate([ar, ai], axis=0).astype(bf16)
            memo[key] = (ar, ai, [i32(ar) ^ i32(ai)])
            return memo[key][2]

        def inv(i):
            yv = jnp.dot(g_v[...], z_v[i % (2 * R)], preferred_element_type=f32)
            if yval:
                memo[("y", i)] = yv
            else:
                y_v[i % (2 * R)] = yv

        def moments(x):
            m = jnp.sum(x, axis=-1, keepdims=True) * (1.0 / D)
            q = jnp.sum(x * x, axis=-1, keepdims=True) * (1.0 / D)
            rstd = lax.rsqrt(jnp.maximum(q - m * m, 0.0) + EPS)
            return m, rstd

        def btok(v):
            vb = jnp.broadcast_to(v, (16, 128))
            return i32(vb[0:8]) ^ i32(vb[8:16])

        def epi_piece(r0, stage=2):
            key = ("epi", r0, stage)
            if key in memo:
                return memo[key][0]
            i = r0 // T
            rs = slice(r0, r0 + 16)
            if stage == 0:
                x = q_v[rs, :].astype(f32)
                if r0 in pace:
                    x = jnp.where(never, jnp.tile(pace.pop(r0), (2, 5)), x)
                m, rstd = moments(x)
                memo[key] = ([btok(rstd) ^ btok(m)], m, rstd, x)
            elif stage == 1:
                epi_piece(r0, 0)
                _, m, rstd, x = memo[("epi", r0, 0)]
                if yval:
                    yc = memo[("y", i)][r0 - i * T:r0 - i * T + 16]
                else:
                    yc = y_v[i % (2 * R), r0 - i * T:r0 - i * T + 16, :]
                y = yc + kv_v[rs, :].astype(f32) * par_v[4, 0:1, :]
                x1 = x + (((x - m) * rstd) * mod_v[0, 0:1, :] + mod_v[1, 0:1, :]) * y
                x1_v[rs, :] = x1
                m2, rstd2 = moments(x1)
                memo[key] = ([btok(rstd2) ^ btok(m2)], x1, m2, rstd2)
            else:
                epi_piece(r0, 1)
                _, x1, m2, rstd2 = memo[("epi", r0, 1)]
                h2 = ((x1 - m2) * rstd2) * mod_v[2, 0:1, :] + mod_v[3, 0:1, :]
                h2_v[rs, :] = h2.astype(bf16)
                memo[key] = (toks16(h2),)
            return memo[key][0]

        def fin_piece(r0):
            rs = slice(r0, r0 + 16)
            o = x1_v[rs, :] + mod_v[4, 0:1, :] * p0_v[rs, :]
            out_v[rs, :] = o.astype(bf16)
            return toks16(o)

        def params():
            sh = shift_v[...].astype(f32)
            for t in range(4):
                par_v[t] = jnp.broadcast_to(sh[t:t + 1, :], (8, D))
            par_v[4] = jnp.broadcast_to(ssmd_v[...].astype(f32).reshape(1, D), (8, D))

        def mods(lo, hi):
            cc = c_v[...].astype(f32)
            sc = (cc * jax.nn.sigmoid(cc)).astype(bf16)
            sc = jnp.broadcast_to(sc, (16, D))
            md = [jnp.dot(sc, wmod_v[:, i * D:(i + 1) * D], preferred_element_type=f32)[0:8, :] for i in range(lo, hi)]
            return md

        def mods_a():
            sa, ca, ga = mods(0, 3)
            mod_v[0] = ga * (1.0 + ca)
            mod_v[1] = ga * sa

        def mods_b():
            sb, cb = mods(3, 5)
            mod_v[2] = 1.0 + cb
            mod_v[3] = sb

        def mods_c():
            (gb,) = mods(5, 6)
            mod_v[4] = gb

        koff = [0]

        def sel16(tok, base):
            r = jnp.where(never, tok, pltpu.bitcast(base, jnp.int32))
            return pltpu.bitcast(r, bf16)

        def dot_w(lhs, rhs, cells):
            if cells and not (interpret and not force_inj):
                M_, K = lhs.shape
                rowp = []
                for rr in range(M_ // 16):
                    cols_ = []
                    for kt in range(K // 128):
                        base = lhs[rr * 16:(rr + 1) * 16, kt * 128:(kt + 1) * 128]
                        cols_.append(sel16(cells[(rr, kt)](), base) if (rr, kt) in cells else base)
                    rowp.append(jnp.concatenate(cols_, axis=1))
                lhs = jnp.concatenate(rowp, axis=0)
            elif cells:
                for key in sorted(cells):
                    cells[key]()
            return jnp.dot(lhs, rhs, preferred_element_type=f32)

        wait("ft", "shift", "ssmd", ("k", 0), ("v", 0))
        params()
        for u_ in range(2):
            wait(("k", u_), ("v", u_))
            for r0 in range(u_ * TM, (u_ + 1) * TM, 16):
                kv_piece(r0)
            wait(("ssmk", u_))
            for b in range(u_ * R, (u_ + 1) * R):
                kspec(b)
                uspec(b)
            wait("g")
            for b in range(u_ * R, (u_ + 1) * R):
                for r in range(T // 8):
                    for c in range(5):
                        mac_piece(b, r, c)
                inv(b)
        wait("c", "wmod_a", ("q", 0), ("q", 1))
        mods_a()
        for r0 in range(0, 2 * TM, 16):
            epi_piece(r0, 1)
        wait("wmod_b")
        mods_b()
        for r0 in range(0, 2 * TM, 16):
            epi_piece(r0, 2)

        def out_copy(m):
            return pltpu.make_async_copy(out_v.at[rows(m), :], out_hbm.at[rows(m), :], sems.at[n_in + m])

        GU_T = 5 * TM // 4
        DN_T = (F // 128) * TM // 4
        SP_T = 5 * 256 // 4

        def run_segment(m, ev, streams, paced=None, hold=False):
            avail = [0] * 4
            job = 0
            cells = []
            jobt = {}
            pace_plan = []
            for i, (kind, n, _) in enumerate(ev):
                njob, dur, nrr = {"g": (5, TM, TM // 16), "u": (5, TM, TM // 16), "d": (F // 128, TM, TM // 16),
                                  "ks": (5, 256, 0), "us": (5, 256, 0), "inv": (10, 128, 0), "mc": (25, 16, 0)}[kind]
                for kt in range(njob):
                    t0 = avail[job % 4]
                    jobt[(i, kt)] = t0
                    avail[job % 4] += dur
                    job += 1
                    cells += [(t0 + 16 * rr, i, rr, kt) for rr in range(nrr)]
            cells.sort()
            used = set()
            assign = {i: {} for i in range(len(ev))}

            def getter(memo, th, k_):
                def get():
                    if not memo:
                        memo.append(th())
                    return memo[0][k_]
                return get

            for thunks, ntoks, wts, (ta, tb) in streams:
                inwin = [c_ for c_ in cells if ta <= c_[0] < tb]
                toks = []
                for p_, th in enumerate(thunks):
                    memo_ = []
                    ntok = ntoks[p_] if isinstance(ntoks, list) else ntoks
                    wt = wts[p_] if isinstance(wts, list) else wts
                    toks += [(getter(memo_, th, k_), wt / ntok) for k_ in range(ntok)]
                wsum = sum(w_ for _, w_ in toks)
                acc_ = 0.0
                for get, w_ in toks:
                    acc_ += w_
                    idx = min(len(inwin) - 1, int(acc_ / wsum * len(inwin)))
                    while inwin[idx] in used:
                        idx = (idx - 1) % len(inwin)
                    used.add(inwin[idx])
                    _, i, rr, kt = inwin[idx]
                    assign[i][(rr, kt)] = get
            if paced is not None and do_pace:
                r0s, ta, tb = paced
                pace_plan = [(ta + (tb - ta) * p_ / len(r0s), r0_) for p_, r0_ in enumerate(r0s)]
            def do_paced(i, last_job, val):
                for (tj, r0_) in list(pace_plan):
                    rr_ = int((tj - jobt[(i, last_job)]) // 16)
                    if rr_ < TM // 16:
                        pace_plan.remove((tj, r0_))
                        rr_ = max(rr_, 0)
                        pace[r0_] = val[rr_ * 16:rr_ * 16 + 8, :]
                        if not etok:
                            epi_piece(r0_, 2)

            for i, (kind, n, _) in enumerate(ev):
                cols = slice(n * NT, (n + 1) * NT)
                if kind == "ks":
                    kspec(n)
                elif kind == "us":
                    uspec(n)
                elif kind == "inv":
                    inv(n)
                elif kind == "mc":
                    mods_c()
                elif kind == "g":
                    gbox[0] = dot_w(h2_v[rows(m), :], wg_v[:, cols], assign[i])
                    do_paced(i, 4, gbox[0])
                elif kind == "u":
                    uval = dot_w(h2_v[rows(m), :], wu_v[:, cols], assign[i])
                    do_paced(i, 4, uval)
                    hh_v[:, cols] = (gbox[0] * uval).astype(bf16)
                elif kind == "d":
                    p = None
                    for w_ in range(KSP):
                        ks_ = slice(w_ * (F // KSP), (w_ + 1) * (F // KSP))
                        nk_ = F // KSP // 128
                        sub = {(rr, kt - w_ * nk_): g_ for (rr, kt), g_ in assign[i].items() if w_ * nk_ <= kt < (w_ + 1) * nk_}
                        pp = dot_w(hh_v[:, ks_], wd_v[ks_, cols], sub)
                        do_paced(i, w_ * nk_ + nk_ - 1, pp)
                        p = pp if p is None else p + pp
                    if hold:
                        p0_v[:, cols] = p
                    else:
                        out_v[rows(m), cols] = (x1_v[rows(m), cols] + mod_v[4, 0:1, cols] * p).astype(bf16)

        gbox = [None]
        held = []

        def gu(ns):
            ev = []
            for n in ns:
                ev += [("g", n, GU_T), ("u", n, GU_T)]
            return ev

        def t_of(ev, kind, last=False):
            tt = 0
            res = None
            for e in ev:
                if e[0] == kind and (res is None or last):
                    res = tt
                tt += e[2]
            return tt if res is None else res

        def kv_stream(mm, win):
            return ([functools.partial(kv_piece, r0) for r0 in range(mm * TM, (mm + 1) * TM, 16)], 5, 1.0, win)

        def mac_stream(mm, win):
            th = []
            for b in range(mm * R, (mm + 1) * R):
                nsub = -(-(b + 1) // tps)
                cuts = [((b + 1) * k_) // nsub for k_ in range(nsub + 1)]
                for r in range(T // 8):
                    for c in range(5):
                        for k_ in range(nsub):
                            th.append(functools.partial(mac_piece, b, r, c, tuple(cuts), k_))
            return (th, 1, 1.0, win)

        def epi_stream(mm, win):
            r0s = list(range(mm * TM, (mm + 1) * TM, 16))
            order = sorted([(p_ + lag * st, st, r0) for p_, r0 in enumerate(r0s) for st in range(3)])
            return ([functools.partial(epi_piece, r0, st) for _, st, r0 in order], [1 if st < 2 else 5 for _, st, r0 in order], [ew[st] for _, st, r0 in order], win)

        def blks(kind, mm):
            return [(kind, b, SP_T) for b in range(mm * R, (mm + 1) * R)]

        pending_out = []
        started = []
        tail_copies = []
        for m in (range(NM) if units is None else units):
            m1, m2 = m + 1, m + 2
            if m == 0:
                for c_ in range(NWC):
                    wait(("wg", c_), ("wu", c_))
                    run_segment(0, gu(range(WCH[c_], WCH[c_ + 1])), [])
                wait(("k", 2), ("v", 2), ("ssmk", 2))
                for r0 in range(2 * TM, 3 * TM, 16):
                    kv_piece(r0)
                for b in range(2 * R, 3 * R):
                    kspec(b); uspec(b)
                for c_ in range(2):
                    wait(("wd", c_))
                    run_segment(0, [("d", n, DN_T) for n in range(DCH[c_], DCH[c_ + 1])], [], hold=True)
                continue
            pre = False
            first = m == 1
            w_kv = w_kv1 * ((1 if m2 < NM else 0) + (1 if pre else 0))
            w_m = 680 * (sum(b + 1 for b in range(m1 * R, (m1 + 1) * R))) if m1 < NM else 0
            w_e = w_e1 if m1 < NM else 0
            t_ffn = 2 * NGU * GU_T + NDN * DN_T
            t_a = t_ffn * w_kv / max(w_kv + w_m + w_e, 1)
            t_b = t_ffn * (w_kv + w_m) / max(w_kv + w_m + w_e, 1)
            ninv = min(NDN - 2, max(0, round((t_b - 2 * NGU * GU_T) / DN_T)))
            if first:
                ninv = 0
            n_us = min(NGU - 2, max(1, int((t_a + GU_T) // (2 * GU_T))))
            ev = []
            n0 = 0
            if first:
                ev += [("mc", 0, 100)]
            if m2 < NM:
                ev += blks("ks", m2)
            for n in range(n0, NGU):
                ev += gu([n])
                if n == n_us and m2 < NM:
                    ev += blks("us", m2)
            for n in range(NDN):
                if n == ninv and m1 < NM:
                    ev += blks("inv", m1)
                ev.append(("d", n, DN_T))
            t_end = t_of(ev, "x")
            streams = []
            t0m = t_m[0]
            if m2 < NM:
                t1k = t_of(ev, "us", True) - 2 * SP_T - GU_T
                streams.append(kv_stream(m2, (0, t1k)))
                if not pre:
                    t0m = max(t0m, t1k * mk_ov)
            if first:
                streams.append(([functools.partial(fin_piece, r0) for r0 in range(0, TM, 16)], 5, 1.0, (t_of(ev, "us", True) + 2 * SP_T, t_of(ev, "inv"))))
            if m1 < NM:
                t_inv_ = t_of(ev, "inv")
                streams.append(mac_stream(m1, (t0m, t_inv_ - t_m[1])))
                if etok:
                    streams.append(epi_stream(m1, (t_inv_ + 2 * SP_T + t_e[0], t_end - t_e[1])))
            pending_out.append(m - 1)
            if first:
                wait(("k", m2), ("v", m2), ("ssmk", m2))
                cut = [i for i, e in enumerate(ev) if e[0] in ("d", "inv")][0]
                evA, evB = [e for e in ev[:cut] if e[0] != "mc"], [("mc", 0, 100)] + ev[cut:]
                tA = t_of(evA, "x")
                run_segment(m, evA, [kv_stream(m2, (0, t_of(evA, "us", True) - 2 * SP_T - GU_T)),
                                     mac_stream(m1, (t_of(evA, "us"), tA - t_m[1]))])
                wait("wmod_c", ("q", m1))
                ti = t_of(evB, "inv")
                pending_out.clear(); pending_out.append(0)
                run_segment(m, evB, [([functools.partial(fin_piece, r0) for r0 in range(0, TM, 16)], 5, 1.0, (200, t_of(evB, "x") - 300)),
                                     epi_stream(m1, (ti + 2 * SP_T + t_e[0], t_of(evB, "x") - t_e[1]))],
                            (list(range(m1 * TM, (m1 + 1) * TM, 16)), ti + 2 * SP_T + pace_w[0], t_of(evB, "x") - pace_w[1]))
                continue
            for mo in pending_out:
                out_copy(mo).start(); started.append(mo)
            pending_out.clear()
            for mm_ in range(m1, min(m2, NM - 1) + 1):
                wait(("k", mm_), ("v", mm_), ("ssmk", mm_), ("q", mm_))
            if m == NM - 1 and tail_split:
                cut = len(ev) - NDN + tail_split
                run_segment(m, ev[:cut], [])
                c_ = tail_split * NT
                ca = pltpu.make_async_copy(out_v.at[rows(m), 0:c_], out_hbm.at[rows(m), 0:c_], sems.at[n_in + NM])
                ca.start()
                run_segment(m, ev[cut:], [])
                cb = pltpu.make_async_copy(out_v.at[rows(m), c_:D], out_hbm.at[rows(m), c_:D], sems.at[n_in + m])
                cb.start()
                tail_copies.extend([ca, cb])
                continue
            paced = None
            if m1 < NM:
                paced = (list(range(m1 * TM, (m1 + 1) * TM, 16)), t_inv_ + 2 * SP_T + pace_w[0], t_end - pace_w[1])
            run_segment(m, ev, streams, paced)
        ms = list(range(NM) if units is None else units)
        for mo in pending_out + ([] if tail_copies else [ms[-1]]):
            out_copy(mo).start(); started.append(mo)
        for mo in started:
            out_copy(mo).wait()
        for cp_ in tail_copies:
            cp_.wait()
        for name, _, _ in plan:
            wait(name)

    def run(A_q, A_k, A_v, A_shift_k, A_ssm_k, A_ssm_D, B_x, B_w_gate, B_w_up, B_w_down, c, w_mod):
        ft, g = _dft_consts()
        any_ = pl.BlockSpec(memory_space=pl.ANY)
        V = pltpu.VMEM
        nsem = 12 + 4 * NM + 2 * NWC + len(DCH) + NM + 1
        out = pl.pallas_call(
            kernel,
            out_shape=jax.ShapeDtypeStruct((S, D), bf16),
            in_specs=[any_] * 13 + [pl.BlockSpec(memory_space=pltpu.SMEM)],
            out_specs=any_,
            scratch_shapes=[
                V((S, D), bf16), V((S, D), bf16), V((S, D), bf16), V((4, D), bf16), V((D, S), bf16), V((D,), bf16),
                V((D, F), bf16), V((D, F), bf16), V((F, D), bf16), V((1, D), bf16), V((D, 6 * D), bf16),
                V((2 * T, T), bf16), V((T, 2 * T), bf16),
                V((2 * NB, 2 * T, D), f32), V((2, 2 * T, D), f32), V((S, D), bf16),
                V((2 * R, 2 * T, D), bf16), V((2 * R, T, D), f32), V((S, D), bf16), V((S, D), f32),
                V((S, D), bf16), V((5, 8, D), f32), V((5, 8, D), f32), V((TM, F), bf16), V((TM, D), f32),
                pltpu.SemaphoreType.DMA((nsem,)),
            ],
            compiler_params=pltpu.CompilerParams(vmem_limit_bytes=vmem_mb * 1024 * 1024, flags=flags),
            interpret=interpret,
        )(A_q.reshape(S, D), A_k.reshape(S, D), A_v.reshape(S, D), A_shift_k.T, A_ssm_k, A_ssm_D,
          B_w_gate, B_w_up, B_w_down, c, w_mod, ft, g, np.zeros((1,), np.int32))
        return out.reshape(1, S, D)
    return run


_run = make_kernel()


@jax.jit
def pallas_adaLN_cond__ssm_conv_h3__glu_gated_bilinear__prompt_kernel(
    A_q: jax.Array,
    A_k: jax.Array,
    A_v: jax.Array,
    A_shift_k: jax.Array,
    A_ssm_k: jax.Array,
    A_ssm_D: jax.Array,
    B_x: jax.Array,
    B_w_gate: jax.Array,
    B_w_up: jax.Array,
    B_w_down: jax.Array,
    c: jax.Array,
    w_mod: jax.Array,
):
    return _run(A_q, A_k, A_v, A_shift_k, A_ssm_k, A_ssm_D, B_x, B_w_gate, B_w_up, B_w_down, c, w_mod)
```
